```python
import jax
import jax.numpy as jnp

def _softmax(x, axis=-1):
    return jax.nn.softmax(x, axis=axis)
def _gelu(x):
    return jax.nn.gelu(x, approximate=True)
def _silu(x):
    return jax.nn.silu(x)
def _sigmoid(x):
    return jax.nn.sigmoid(x)
def _layernorm(x, axis=-1, eps=1e-5):
    m = jnp.mean(x, axis=axis, keepdims=True)
    v = jnp.var(x, axis=axis, keepdims=True)
    return (x - m) / jnp.sqrt(v + eps)
def _scatter_add(tgt, idx, src, axis=0):
    return tgt.at[idx].add(src)
def _segment_sum(src, seg, n):
    return jax.ops.segment_sum(src, seg, n)
class _Rng:
    def __init__(self, key):
        self._k = key
    def _next(self):
        self._k, sub = jax.random.split(self._k)
        return sub
    def normal(self, shape):
        return jax.random.normal(self._next(), shape, dtype=jnp.bfloat16)
    def randint(self, lo, hi, shape):
        return jax.random.randint(self._next(), shape, lo, hi, dtype=jnp.int32)
    def uniform(self, shape, lo=0.0, hi=1.0):
        return jax.random.uniform(self._next(), shape, jnp.bfloat16, lo, hi)
    def permutation(self, n):
        return jax.random.permutation(self._next(), n)


kernel_name = 'gated_mix__ssm_conv_h3__sliding_local_dilated__prompt'

def setup_inputs():
    _rng = _Rng(jax.random.key(int.from_bytes(__import__("os").urandom(4), "little")))
    _w = (lambda a: (lambda t: t.astype(jnp.bfloat16) if jnp.issubdtype(t.dtype, jnp.floating) else t)(jnp.asarray(a)))
    def _A_setup():
        B, S, D = 1, 2048, 640
        ks = 4
        return {
            "q": _w((lambda *s: _rng.normal(s) * 0.05)(B, S, D)),
            "k": _w((lambda *s: _rng.normal(s) * 0.05)(B, S, D)),
            "v": _w((lambda *s: _rng.normal(s) * 0.05)(B, S, D)),
            "shift_k": _w((lambda *s: _rng.normal(s) * 0.05)(D, ks) * 0.5),
            "ssm_k": _w((lambda *s: _rng.normal(s) * 0.05)(D, S) * (1.0 / S ** 0.5)),
            "ssm_D": _w((lambda *s: _rng.normal(s) * 0.05)(D)),
        }
    _A_in = _A_setup()

    def _B_setup():
        B, S, D = 1, 2048, 640
        return {
            "x": _w((lambda *s: _rng.normal(s) * 0.05)(B, S, D)),
            "wqkv": _w((lambda *s: _rng.normal(s) * 0.05)(D, 3 * D)),
            "wo": _w((lambda *s: _rng.normal(s) * 0.05)(D, D)),
        }
    _B_in = _B_setup()

    return {
        "A_q": _A_in["q"],
        "A_k": _A_in["k"],
        "A_v": _A_in["v"],
        "A_shift_k": _A_in["shift_k"],
        "A_ssm_k": _A_in["ssm_k"],
        "A_ssm_D": _A_in["ssm_D"],
        "B_x": _B_in["x"],
        "B_wqkv": _B_in["wqkv"],
        "B_wo": _B_in["wo"],
        "gate_w": _w((lambda *s: _rng.normal(s) * 0.05)(640)),
    }

def reference(A_q, A_k, A_v, A_shift_k, A_ssm_k, A_ssm_D, B_x, B_wqkv, B_wo, gate_w):
    def _A_ref(q, k, v, shift_k, ssm_k, ssm_D):
        B, S, D = q.shape
        ks = shift_k.shape[-1]
        k_pad = jnp.pad(k, ((0, 0), (ks - 1, 0), (0, 0)))
        k_shift = jnp.zeros_like(k)
        for t in range(ks):
            k_shift = k_shift + k_pad[:, t:t + S, :] * shift_k[:, ks - 1 - t][None, None, :]
        kv = k_shift * v
        L = 2 * S
        kv_pad = jnp.pad(kv, ((0, 0), (0, S), (0, 0)))
        kf_pad = jnp.pad(ssm_k, ((0, 0), (0, S)))
        kv_f = (lambda x, axes=(-2,-1): jnp.fft.rfft2(x.astype(jnp.float32), axes=axes))(kv_pad[:, None, :, :], axes=(1, 2))
        kf_f = (lambda x, axes=(-2,-1): jnp.fft.rfft2(x.astype(jnp.float32), axes=axes))(kf_pad[:, None, :], axes=(1, 2))
        kf_f = (lambda x, *d: x.transpose(*d))(kf_f, 1, 2, 0)
        y_f = kv_f * kf_f[None, :, :, :]
        y = (lambda x, s, axes=(-2,-1): jnp.fft.irfft2(x, s=s, axes=axes).astype(jnp.bfloat16))(y_f, (1, L), axes=(1, 2))[:, 0, :S, :]
        y = y + kv * ssm_D[None, None, :]
        return q * y

    def _B_ref(x, wqkv, wo):
        B, S, D = x.shape
        H = 32; Dh = D // H
        W, dil = 8, 2
        qkv = (lambda x, *d: x.transpose(*d))((x @ wqkv).reshape(B, S, 3, H, Dh), 2, 0, 3, 1, 4)
        q, k, v = qkv[0], qkv[1], qkv[2]
        scale = Dh ** -0.5
        pos = jnp.arange(S)
        off = jnp.arange(W) * dil
        idx = pos[:, None] - off[None, :]
        mask = idx >= 0
        idx_c = jnp.where(mask, idx, 0).reshape(-1)
        kg = k[:, :, idx_c, :].reshape(B, H, S, W, Dh)
        vg = v[:, :, idx_c, :].reshape(B, H, S, W, Dh)
        logits = jnp.einsum("bhsd,bhswd->bhsw", q, kg) * scale
        logits = jnp.where(mask[None, None, :, :], logits, -1e9)
        attn = _softmax(logits, axis=-1)
        o = jnp.einsum("bhsw,bhswd->bhsd", attn, vg)
        return (lambda x, *d: x.transpose(*d))(o, 0, 2, 1, 3).reshape(B, S, D) @ wo

    x = A_q
    g = _sigmoid((x * gate_w).sum(-1, keepdims=True))
    a = _A_ref(x, A_k, A_v, A_shift_k, A_ssm_k, A_ssm_D)
    b = _B_ref(x, B_wqkv, B_wo)
    return g * a + (1 - g) * b
```

```python
import jax
import jax.numpy as jnp
import numpy as np
from jax import lax
from jax.experimental import pallas as pl
from jax.experimental.pallas import tpu as pltpu

S = 2048
D = 640
NH = 32
DH = D // NH
WIN = 8
DIL = 2
KS = 4
L = 128
NC = D // L
NCH = S // L
NF8 = L // 8
HALO = 16
RT = 256
NRT = S // RT
F32 = jnp.float32
BF16 = jnp.bfloat16


def _dft_matrices():
    n = np.arange(L)
    k = np.arange(L)
    ang = 2.0 * np.pi * (((4 * k[:, None] + 1) * n[None, :]) % (4 * L)) / (4 * L)
    fwd = np.stack([np.cos(ang).reshape(NF8, 8, L), -np.sin(ang).reshape(NF8, 8, L)], axis=1)
    fwd = fwd.reshape(2 * L, L)
    inv = fwd.T / L
    return fwd.astype(BF16), np.ascontiguousarray(inv).astype(BF16)


_FWD, _INV = _dft_matrices()
_NT = (((1,), (1,)), ((), ()))


def _kernel(q_hbm, k_hbm, v_hbm, shift_ref, hk_hbm, ssmd_ref, w_hbm, wo_hbm, gate_ref,
            fwd_ref, inv_ref, out_hbm,
            q_s, k_s, v_s, hk_s, w_s, wo_s, wp_s, wop_s, tmp_s, kf_s, par_s,
            xf_s, hf_s, z_s, qf_s, kk_s, vv_s, o_s, b_s, out_s, in_sem, out_sem):
    hk_cp = [pltpu.make_async_copy(hk_hbm.at[pl.ds(c * L, L), :], hk_s.at[c], in_sem.at[c])
             for c in range(NC)]
    w_cp = pltpu.make_async_copy(w_hbm, w_s, in_sem.at[NC])
    wo_cp = pltpu.make_async_copy(wo_hbm, wo_s, in_sem.at[NC + 1])
    q_cp = pltpu.make_async_copy(q_hbm, q_s, in_sem.at[NC + 2])
    k_cp = [pltpu.make_async_copy(k_hbm.at[:, pl.ds(c * L, L)], k_s.at[c], in_sem.at[NC + 3 + c])
            for c in range(NC)]
    v_cp = [pltpu.make_async_copy(v_hbm.at[:, pl.ds(c * L, L)], v_s.at[c], in_sem.at[2 * NC + 3 + c])
            for c in range(NC)]
    for cp in hk_cp:
        cp.start()
    w_cp.start()
    for c in range(NC):
        k_cp[c].start()
        v_cp[c].start()
    wo_cp.start()
    q_cp.start()

    taps = shift_ref[...].astype(F32)
    ssmd = ssmd_ref[...].astype(F32)
    for c in range(NC):
        par_s[c, pl.ds(0, KS), :] = taps[:, c * L:(c + 1) * L]
        par_s[c, pl.ds(KS, 1), :] = ssmd[:, c * L:(c + 1) * L]
    kf_s[pl.ds(0, 8), :] = jnp.zeros((8, L), F32)
    for c in range(NC):
        kk_s[c, pl.ds(0, HALO), :] = jnp.zeros((HALO, L), F32)
        vv_s[c, pl.ds(0, HALO), :] = jnp.zeros((HALO, L), F32)

    def filter_dft(c):
        for m in range(NCH):
            hf_s[c * NCH + m] = lax.dot_general(
                fwd_ref[...], hk_s[c, :, m * L:(m + 1) * L], _NT, preferred_element_type=F32)

    def signal_dft(c):
        kf_s[pl.ds(8, S), :] = k_s[c].astype(F32)
        tap = [par_s[c, pl.ds(t, 1), :] for t in range(KS)]
        for j in range(NCH):
            ks = kf_s[pl.ds(8 + j * L, L), :] * tap[0]
            for t in range(1, KS):
                ks = ks + kf_s[pl.ds(8 + j * L - t, L), :] * tap[t]
            kv = ks * v_s[c, pl.ds(j * L, L), :].astype(F32)
            xf_s[c * NCH + j] = jnp.dot(fwd_ref[...], kv.astype(BF16), preferred_element_type=F32)

    def head_major_to_dim_major():
        return jnp.concatenate([tmp_s[pl.ds(d, NH, stride=DH), :] for d in range(DH)], axis=0)

    def permute_wqkv(rb):
        rows = pl.ds(pl.multiple_of(rb * L, L), L)
        for p in range(3):
            tmp_s[...] = w_s[rows, p * D:(p + 1) * D].astype(F32).T
            wp_s[rows, p * D:(p + 1) * D] = head_major_to_dim_major().T.astype(BF16)

    def permute_wo():
        for c in range(NC):
            tmp_s[...] = wo_s[:, c * L:(c + 1) * L].astype(F32)
            wop_s[:, c * L:(c + 1) * L] = head_major_to_dim_major().astype(BF16)

    def causal_conv(a, b):
        out = []
        for i in range(NCH):
            acc = a[i] * b[0]
            for j in range(1, i + 1):
                acc = acc + a[i - j] * b[j]
            out.append(acc)
        return out

    def spectral_unit(u):
        c = u // NF8
        r = pl.multiple_of((u % NF8) * 16, 16)
        re, im = pl.ds(r, 8), pl.ds(r + 8, 8)
        base = c * NCH
        hr = [hf_s[base + m, re, :] for m in range(NCH)]
        hi = [hf_s[base + m, im, :] for m in range(NCH)]
        hr[0] = hr[0] + par_s[c, pl.ds(KS, 1), :]
        a = [hr[0]] + [hr[m] - hi[m - 1] for m in range(1, NCH)]
        b = [hi[0]] + [hi[m] + hr[m - 1] for m in range(1, NCH)]
        xr = [xf_s[base + j, re, :] for j in range(NCH)]
        xi = [xf_s[base + j, im, :] for j in range(NCH)]
        k1 = causal_conv(a, [xr[j] + xi[j] for j in range(NCH)])
        k3 = causal_conv([a[m] + b[m] for m in range(NCH)], xi)
        zr = [k1[i] - k3[i] for i in range(NCH)]
        k2 = causal_conv([b[m] - a[m] for m in range(NCH)], xr)
        for i in range(NCH):
            z_s[base + i, pl.ds(r, 16), :] = jnp.concatenate(
                [zr[i], k1[i] + k2[i]], axis=0).astype(BF16)

    qscale = float(DH ** -0.5 * np.log2(np.e))

    def project(t):
        r0 = pl.multiple_of(t * RT, RT)
        x = q_s[pl.ds(r0, RT), :]
        for p, dst in enumerate((qf_s, kk_s, vv_s)):
            y = jnp.dot(x, wp_s[:, p * D:(p + 1) * D], preferred_element_type=F32)
            for c in range(NC):
                yc = y[:, c * L:(c + 1) * L]
                if p == 0:
                    dst[c, pl.ds(r0, RT), :] = yc * qscale
                else:
                    dst[c, pl.ds(r0 + HALO, RT), :] = yc

    def attend(r0, masked):
        n = 16
        qs = [qf_s[c, pl.ds(r0, n), :] for c in range(NC)]
        logits = []
        for w in range(WIN):
            rows = pl.ds(r0 + HALO - DIL * w, n)
            acc = qs[0] * kk_s[0, rows, :]
            for c in range(1, NC):
                acc = acc + qs[c] * kk_s[c, rows, :]
            acc = acc + pltpu.roll(acc, 2 * NH, 1)
            acc = acc + pltpu.roll(acc, NH, 1)
            if masked and w > 0:
                pos = r0 + lax.broadcasted_iota(jnp.int32, (n, L), 0)
                acc = jnp.where(pos >= DIL * w, acc, -1e9)
            logits.append(acc)
        m = logits[0]
        for w in range(1, WIN):
            m = jnp.maximum(m, logits[w])
        e = [jnp.exp2(l - m) for l in logits]
        den = e[0]
        for w in range(1, WIN):
            den = den + e[w]
        inv = 1.0 / den
        for c in range(NC):
            acc = e[0] * vv_s[c, pl.ds(r0 + HALO, n), :]
            for w in range(1, WIN):
                acc = acc + e[w] * vv_s[c, pl.ds(r0 + HALO - DIL * w, n), :]
            o_s[pl.ds(r0, n), c * L:(c + 1) * L] = (acc * inv).astype(BF16)

    def out_project(t):
        rows = pl.ds(pl.multiple_of(t * RT, RT), RT)
        b_s[rows, :] = jnp.dot(o_s[rows, :], wop_s[...], preferred_element_type=F32)

    def out_copy(i):
        rows = pl.ds(pl.multiple_of(i * L, L), L)
        return pltpu.make_async_copy(out_s.at[rows, :], out_hbm.at[rows, :], out_sem.at[i])

    def finish(i):
        rows = pl.ds(pl.multiple_of(i * L, L), L)
        x = q_s[rows, :].astype(F32)
        g = jax.nn.sigmoid(jnp.sum(x * gate_ref[...].astype(F32), axis=-1, keepdims=True))
        for c in range(NC):
            cols = slice(c * L, (c + 1) * L)
            y = jnp.dot(inv_ref[...], z_s[c * NCH + i], preferred_element_type=F32)
            out_s[rows, cols] = (g * (x[:, cols] * y) + (1.0 - g) * b_s[rows, cols]).astype(BF16)

    for c in range(NC):
        hk_cp[c].wait()

    @pl.loop(0, NC)
    def _(c):
        filter_dft(c)

    w_cp.wait()

    @pl.loop(0, NC)
    def _(rb):
        permute_wqkv(rb)

    for c in range(NC):
        k_cp[c].wait()
        v_cp[c].wait()

    @pl.loop(0, NC)
    def _(c):
        signal_dft(c)

    wo_cp.wait()
    permute_wo()
    q_cp.wait()
    project(0)

    units = NC * NF8 // NRT

    @pl.loop(0, NRT)
    def _(t):
        r0 = pl.multiple_of(t * RT, RT)
        for s in range(RT // 16):
            attend(r0 + s * 16, masked=(s == 0))
        for s in range(units):
            spectral_unit(t * units + s)
        project(jnp.minimum(t + 1, NRT - 1))
        out_project(t)

    @pl.loop(0, NCH)
    def _(i):
        finish(i)
        out_copy(i).start()

    for i in range(NCH):
        out_copy(i).wait()


@jax.jit
def pallas_gated_mix__ssm_conv_h3__sliding_local_dilated__prompt_kernel(
    A_q: jax.Array,
    A_k: jax.Array,
    A_v: jax.Array,
    A_shift_k: jax.Array,
    A_ssm_k: jax.Array,
    A_ssm_D: jax.Array,
    B_x: jax.Array,
    B_wqkv: jax.Array,
    B_wo: jax.Array,
    gate_w: jax.Array,
):
    del B_x
    hbm = pl.BlockSpec(memory_space=pl.ANY)
    vmem = pl.BlockSpec(memory_space=pltpu.VMEM)
    out = pl.pallas_call(
        _kernel,
        out_shape=jax.ShapeDtypeStruct((S, D), BF16),
        in_specs=[hbm, hbm, hbm, vmem, hbm, vmem, hbm, hbm, vmem, vmem, vmem],
        out_specs=hbm,
        scratch_shapes=[
            pltpu.VMEM((S, D), BF16),
            pltpu.VMEM((NC, S, L), BF16),
            pltpu.VMEM((NC, S, L), BF16),
            pltpu.VMEM((NC, L, S), BF16),
            pltpu.VMEM((D, 3 * D), BF16),
            pltpu.VMEM((D, D), BF16),
            pltpu.VMEM((D, 3 * D), BF16),
            pltpu.VMEM((D, D), BF16),
            pltpu.VMEM((D, L), F32),
            pltpu.VMEM((8 + S, L), F32),
            pltpu.VMEM((NC, 8, L), F32),
            pltpu.VMEM((NC * NCH, 2 * L, L), F32),
            pltpu.VMEM((NC * NCH, 2 * L, L), F32),
            pltpu.VMEM((NC * NCH, 2 * L, L), BF16),
            pltpu.VMEM((NC, S, L), F32),
            pltpu.VMEM((NC, HALO + S, L), F32),
            pltpu.VMEM((NC, HALO + S, L), F32),
            pltpu.VMEM((S, D), BF16),
            pltpu.VMEM((S, D), F32),
            pltpu.VMEM((S, D), BF16),
            pltpu.SemaphoreType.DMA((3 * NC + 3,)),
            pltpu.SemaphoreType.DMA((NCH,)),
        ],
        compiler_params=pltpu.CompilerParams(vmem_limit_bytes=100 * 1024 * 1024),
    )(
        A_q.reshape(S, D), A_k.reshape(S, D), A_v.reshape(S, D),
        A_shift_k.T, A_ssm_k, A_ssm_D.reshape(1, D), B_wqkv, B_wo, gate_w.reshape(1, D),
        _FWD, _INV,
    )
    return out.reshape(1, S, D)
```

```python
import jax
import jax.numpy as jnp
import numpy as np
from jax import lax
from jax.experimental import pallas as pl
from jax.experimental.pallas import tpu as pltpu

S = 2048
D = 640
NH = 32
DH = D // NH
WIN = 8
DIL = 2
KS = 4
L = 128
NC = D // L
NCH = S // L
NF8 = L // 8
HALO = 16
RT = 256
NRT = S // RT
import os
REDUCE = os.environ.get('REDUCE', 'xlu')
AR = int(os.environ.get('AR', 16))
NT_GROUP = int(os.environ.get('NTG', 1))
RT = int(os.environ.get('RT', 256)); NRT = S // RT
SB = int(os.environ.get('SB', 4))
XF0 = 0
HF0 = XF0 + NC * NCH * 3 * L
XTOK = HF0 + NC * NCH * 3 * L
F_ROWS = XTOK + 8 * NRT
PT = HALO + RT
PTOK = 3 * NC * PT
P_ROWS = PTOK + 8 * NRT
SR = int(os.environ.get('SR', 32)); LAG = int(os.environ.get('LAG', 3)); PRE = float(os.environ.get('PRE', 0.015)); POST = float(os.environ.get('POST', 0.0))
U_PHASE = int(os.environ.get('UP', 11)); U_FIRST = NC * NF8 - (NRT - 2) * U_PHASE
F32 = jnp.float32
BF16 = jnp.bfloat16


def _dft_matrices():
    n = np.arange(L)
    k = np.arange(L)
    ang = 2.0 * np.pi * (((4 * k[:, None] + 1) * n[None, :]) % (4 * L)) / (4 * L)
    fwd = np.concatenate([np.cos(ang), -np.sin(ang)], axis=0)
    inv = fwd.reshape(2, NF8, 8, L).transpose(1, 0, 2, 3).reshape(2 * L, L).T / L
    return fwd.astype(BF16), np.ascontiguousarray(inv).astype(BF16)


_FWD, _INV = _dft_matrices()
_SAME_HEAD = (np.arange(L)[:, None] % NH == np.arange(L)[None, :] % NH).astype(BF16)
_NT = (((1,), (1,)), ((), ()))


def _kernel(q_hbm, k_hbm, v_hbm, shift_ref, hk_hbm, ssmd_ref, w_hbm, wo_hbm, gate_ref,
            fwd_ref, inv_ref, zero_ref, out_hbm,
            q_s, k_s, v_s, hk_s, w_s, wo_s, wp_s, wop_s, tmp_s, kf_s, par_s,
            z_s, f_s, pa_s, pb_s, o_s, b_s, lg_s, out_s, in_sem, out_sem):
    def hk_cp(c):
        rows = pl.ds(pl.multiple_of(c * L, L), L)
        return pltpu.make_async_copy(hk_hbm.at[rows, :], hk_s.at[c], in_sem.at[c])

    def w_cp(c):
        rows = pl.ds(pl.multiple_of(c * L, L), L)
        return pltpu.make_async_copy(w_hbm.at[rows, :], w_s.at[c], in_sem.at[NC + c])

    def col_cp(src, dst, c, r0, n, sem):
        return pltpu.make_async_copy(src.at[pl.ds(r0, n), pl.ds(c * L, L)],
                                     dst.at[c, pl.ds(r0, n), :], in_sem.at[sem * NC + c])

    k_cp = [col_cp(k_hbm, k_s, c, 0, S, 2) for c in range(NC)]
    v_cp = [col_cp(v_hbm, v_s, c, 0, S, 3) for c in range(NC)]
    q_cp = [[col_cp(q_hbm, q_s, c, r0, n, 4 + i) for c in range(NC)]
            for i, (r0, n) in enumerate(((0, RT), (RT, RT), (2 * RT, S - 2 * RT)))]
    wo_cp = pltpu.make_async_copy(wo_hbm, wo_s, in_sem.at[7 * NC])
    for c in range(NC):
        hk_cp(c).start()
        w_cp(c).start()
    for cp in q_cp[0]:
        cp.start()
    for c in range(NC):
        k_cp[c].start()
        v_cp[c].start()
    for cp in q_cp[1] + [wo_cp] + q_cp[2]:
        cp.start()

    taps = shift_ref[...].astype(F32)
    ssmd = ssmd_ref[...].astype(F32).reshape(1, D)
    gate = gate_ref[...].astype(F32).reshape(1, D)
    for c in range(NC):
        par_s[c, pl.ds(0, KS), :] = taps[:, c * L:(c + 1) * L]
        par_s[c, pl.ds(KS, 1), :] = ssmd[:, c * L:(c + 1) * L]
        par_s[c, pl.ds(KS + 1, 1), :] = gate[:, c * L:(c + 1) * L]
    kf_s[pl.ds(0, 8), :] = jnp.zeros((8, L), F32)
    for n in range(NC, 3 * NC):
        pa_s[pl.ds(n * PT, HALO), :] = jnp.zeros((HALO, L), F32)

    def filter_dft(c):
        prev = None
        for m in range(NCH):
            h = lax.dot_general(
                fwd_ref[...], hk_s[c, :, m * L:(m + 1) * L], _NT, preferred_element_type=F32)
            hr, hi = h[:L], h[L:]
            if m == 0:
                hr = hr + par_s[c, pl.ds(KS, 1), :]
                a, b = hr, hi
            else:
                a, b = hr - prev[1], hi + prev[0]
            prev = (hr, hi)
            f_s[pl.ds(HF0 + (c * NCH + m) * 3 * L + 0, L), :] = a
            f_s[pl.ds(HF0 + (c * NCH + m) * 3 * L + L, L), :] = b - a
            f_s[pl.ds(HF0 + (c * NCH + m) * 3 * L + 2 * L, L), :] = a + b

    def signal_dft(c):
        kf_s[pl.ds(8, S), :] = k_s[c].astype(F32)
        tap = [par_s[c, pl.ds(t, 1), :] for t in range(KS)]
        for j in range(NCH):
            ks = kf_s[pl.ds(8 + j * L, L), :] * tap[0]
            for t in range(1, KS):
                ks = ks + kf_s[pl.ds(8 + j * L - t, L), :] * tap[t]
            kv = ks * v_s[c, pl.ds(j * L, L), :].astype(F32)
            x = jnp.dot(fwd_ref[...], kv.astype(BF16), preferred_element_type=F32)
            f_s[pl.ds(XF0 + (c * NCH + j) * 3 * L + 0, L), :] = x[:L] + x[L:]
            f_s[pl.ds(XF0 + (c * NCH + j) * 3 * L + L, 2 * L), :] = x
            yield x[2 * L - 8:]

    def head_major_to_dim_major(p):
        return jnp.concatenate([tmp_s[p, pl.ds(d, NH, stride=DH), :] for d in range(DH)], axis=0)

    def permute_wqkv(rb):
        for p in range(3):
            tmp_s[p] = w_s[rb, :, p * D:(p + 1) * D].astype(F32).T
            wt = head_major_to_dim_major(p).astype(BF16)
            for c in range(NC):
                wp_s[(p * NC + c) * NC + rb] = wt[c * L:(c + 1) * L]

    def permute_wo():
        for c in range(NC):
            tmp_s[c % 3] = wo_s[:, c * L:(c + 1) * L].astype(F32)
            wt = head_major_to_dim_major(c % 3).astype(BF16)
            for rb in range(NC):
                wop_s[c * NC + rb] = wt[rb * L:(rb + 1) * L]

    def spectral(u):
        c, f8 = u // NF8, u % NF8

        def conv(part, i0, acc, sign):
            row = c * NCH * 3 * L + part * L + f8 * 8
            h = {}
            for j in range(i0 + SB):
                x = f_s[pl.ds(pl.multiple_of(XF0 + row + j * 3 * L, 8), 8), :]
                for i in range(max(i0, j), i0 + SB):
                    if i - j not in h:
                        h[i - j] = f_s[pl.ds(pl.multiple_of(HF0 + row + (i - j) * 3 * L, 8), 8), :]
                    p = h[i - j] * x
                    prev = acc[i - i0]
                    acc[i - i0] = p if prev is None else (prev + p if sign > 0 else prev - p)
                yield 2 * (i0 + SB - max(i0, j))

        for i0 in range(0, NCH, SB):
            k1 = [None] * SB
            yield from conv(0, i0, k1, 1)
            zr = list(k1)
            yield from conv(2, i0, zr, -1)
            yield from conv(1, i0, k1, 1)
            for i in range(SB):
                z_s[c * NCH + i0 + i, pl.ds(pl.multiple_of(f8 * 16, 16), 16), :] = jnp.concatenate(
                    [zr[i], k1[i]], axis=0).astype(BF16)

    qscale = float(DH ** -0.5 * np.log2(np.e))

    def attention(r0, src):
        def shifted(base, c, g, w):
            return src[pl.ds((base + c) * PT + HALO + 8 * g - DIL * w, 8), :]

        def scores(g):
            qs = [shifted(0, c, g, 0) for c in range(NC)]
            for w in range(WIN):
                acc = qs[0] * shifted(NC, 0, g, w)
                for c in range(1, NC):
                    acc = acc + qs[c] * shifted(NC, c, g, w)
                acc = acc + pltpu.roll(acc, 2 * NH, 1)
                acc = acc + pltpu.roll(acc, NH, 1)
                if 8 * g < DIL * w:
                    pos = r0 + 8 * g + lax.broadcasted_iota(jnp.int32, (8, L), 0)
                    acc = jnp.where(pos >= DIL * w, acc, -1e9)
                lg_s[pl.ds(8 * (g * WIN + w), 8), :] = acc
                yield 11

        def mix(g):
            logits = [lg_s[pl.ds(8 * (g * WIN + w), 8), :] for w in range(WIN)]
            m = logits[0]
            for w in range(1, WIN):
                m = jnp.maximum(m, logits[w])
            e = [jnp.exp2(l - m) for l in logits]
            den = e[0]
            for w in range(1, WIN):
                den = den + e[w]
            inv = 1.0 / den
            yield 30
            for c in range(NC):
                acc = e[0] * shifted(2 * NC, c, g, 0)
                for w in range(1, WIN):
                    acc = acc + e[w] * shifted(2 * NC, c, g, w)
                acc = acc * inv
                if g % 2 == 0:
                    half[c] = acc
                else:
                    o_s[c, pl.ds(r0 + 8 * (g - 1), 16), :] = jnp.concatenate(
                        [half[c], acc], axis=0).astype(BF16)
                yield 16

        groups = RT // 8
        half = [None] * NC
        for g in range(groups + LAG):
            if g < groups:
                yield from scores(g)
            if g >= LAG:
                yield from mix(g - LAG)

    def projections(jobs):
        def dot(job, ks):
            lhs_ref, r0, w_ref, n = job[:4]
            lhs = jnp.concatenate([lhs_ref[c, pl.ds(r0, RT), :] for c in ks], axis=1)
            if w_ref is wp_s:
                w = jnp.concatenate([w_ref[n * NC + c] for c in ks], axis=1)
                return lax.dot_general(lhs, w, _NT, preferred_element_type=F32)
            w = jnp.concatenate([w_ref[n * NC + c] for c in ks], axis=0)
            return jnp.dot(lhs, w, preferred_element_type=F32)

        rounds = []
        for g in range(0, len(jobs), 4):
            rounds += [[(job, dot(job, range(NC - 1)))] for job in jobs[g:g + 4]]
            rounds.append([(job, dot(job, [NC - 1])) for job in jobs[g:g + 4]])

        def stores():
            for i, rnd in enumerate(rounds):
                last = i % 5 == 4 or i == len(rounds) - 1
                for r in range(0, RT, SR):
                    for (_, _, _, _, dst, row, scale), y in rnd:
                        rows = pl.ds(row + r, SR)
                        yr = y[r:r + SR]
                        if last:
                            yr = yr + dst[rows, :]
                            yr = yr if scale is None else yr * scale
                        dst[rows, :] = yr
                    yield yr[SR - 8:]

        return stores(), len(rounds) * RT // SR

    def qkv_jobs(r0, dst):
        return [(q_s, r0, wp_s, n, dst, n * PT + HALO, qscale if n < NC else None)
                for n in range(3 * NC)]

    def out_jobs(r0):
        return [(o_s, r0, wop_s, n, b_s, n * S + r0, None) for n in range(NC)]

    def chain(*gens):
        for g in gens:
            yield from g

    def weave(lead, steps, followers):
        done = [0] * len(followers)

        def advance(frac, anchor):
            for i, (gen, total, pace) in enumerate(followers):
                if anchor is not None and done[i] < frac * total:
                    pace(anchor)
                while done[i] < frac * total:
                    done[i] += next(gen)

        advance(PRE / (1 + PRE + POST), None)
        for i, anchor in enumerate(lead):
            advance(min((PRE + (i + 1) / steps) / (1 + PRE + POST), 0.9999), anchor)
        for gen, _, _ in followers:
            for _ in gen:
                pass

    def out_copy(i):
        rows = pl.ds(i * L, L)
        return pltpu.make_async_copy(out_s.at[rows, :], out_hbm.at[rows, :], out_sem.at[i])

    def finish(i):
        rows = pl.ds(i * L, L)
        x = [q_s[c, rows, :].astype(F32) for c in range(NC)]
        dot = x[0] * par_s[0, pl.ds(KS + 1, 1), :]
        for c in range(1, NC):
            dot = dot + x[c] * par_s[c, pl.ds(KS + 1, 1), :]
        g = jax.nn.sigmoid(jnp.sum(dot, axis=-1, keepdims=True))
        for c in range(NC):
            y = jnp.dot(inv_ref[...], z_s[c * NCH + i], preferred_element_type=F32)
            b = b_s[pl.ds(c * S + i * L, L), :]
            out_s[rows, c * L:(c + 1) * L] = (g * (x[c] * y) + (1.0 - g) * b).astype(BF16)
            yield y[L - 8:]

    attn_work = (RT // 8) * (11 * WIN + 30 + 16 * NC)

    def attn_stream(t, src):
        def pace(y):
            src[pl.ds(pl.multiple_of(PTOK + anywhere, 8), 8), :] = y
        return attention(pl.multiple_of(t * RT, RT), src), attn_work, pace

    def spec_stream(u0, n):
        def pace(y):
            f_s[pl.ds(pl.multiple_of(XTOK + anywhere, 8), 8), :] = y
        return chain(*[spectral(u0 + i) for i in range(n)]), n * 3 * NCH * (NCH + 1), pace

    def carry_halo(src, dst):
        for n in range(NC, 3 * NC):
            dst[pl.ds(n * PT, HALO), :] = src[pl.ds(n * PT + RT, HALO), :]

    anywhere = zero_ref[0]

    @pl.loop(0, NC)
    def _(c):
        hk_cp(c).wait()
        w_cp(c).wait()
        filter_dft(c)
        permute_wqkv(c)

    for cp in q_cp[0]:
        cp.wait()
    weave(*projections(qkv_jobs(0, pa_s)), [])

    for c in range(NC):
        k_cp[c].wait()
        v_cp[c].wait()
    weave(chain(*[signal_dft(c) for c in range(NC)]), NC * NCH, [attn_stream(0, pa_s)])

    for cp in q_cp[1] + [wo_cp]:
        cp.wait()
    permute_wo()
    carry_halo(pa_s, pb_s)
    weave(*projections(qkv_jobs(RT, pb_s)), [spec_stream(0, U_FIRST)])

    for cp in q_cp[2]:
        cp.wait()

    def phase(t, cur, nxt):
        row = lambda i: pl.multiple_of(i * RT, RT)
        carry_halo(cur, nxt)
        weave(*projections(out_jobs(row(t - 1)) + qkv_jobs(row(t + 1), nxt)),
              [attn_stream(t, cur), spec_stream(U_FIRST + (t - 1) * U_PHASE, U_PHASE)])

    @pl.loop(0, (NRT - 2) // 2)
    def _(i):
        phase(2 * i + 1, pb_s, pa_s)
        phase(2 * i + 2, pa_s, pb_s)

    early = (S - 2 * RT) // L
    lead, steps = projections(out_jobs(S - 2 * RT))
    weave(chain(lead, *[finish(i) for i in range(early)]), steps + early * NC,
          [attn_stream(NRT - 1, pb_s)])
    for i in range(early):
        out_copy(i).start()
    lead, steps = projections(out_jobs(S - RT))
    weave(chain(*[finish(i) for i in range(early, early + RT // L)], lead,
                *[finish(i) for i in range(early + RT // L, NCH)]), 1, [])
    for i in range(early, NCH):
        out_copy(i).start()
    for i in range(NCH):
        out_copy(i).wait()


@jax.jit
def pallas_gated_mix__ssm_conv_h3__sliding_local_dilated__prompt_kernel(
    A_q: jax.Array,
    A_k: jax.Array,
    A_v: jax.Array,
    A_shift_k: jax.Array,
    A_ssm_k: jax.Array,
    A_ssm_D: jax.Array,
    B_x: jax.Array,
    B_wqkv: jax.Array,
    B_wo: jax.Array,
    gate_w: jax.Array,
):
    del B_x
    hbm = pl.BlockSpec(memory_space=pl.ANY)
    vmem = pl.BlockSpec(memory_space=pltpu.VMEM)
    smem = pl.BlockSpec(memory_space=pltpu.SMEM)
    out = pl.pallas_call(
        _kernel,
        out_shape=jax.ShapeDtypeStruct((S, D), BF16),
        in_specs=[hbm, hbm, hbm, vmem, hbm, vmem, hbm, hbm, vmem, vmem, vmem, smem],
        out_specs=hbm,
        scratch_shapes=[
            pltpu.VMEM((NC, S, L), BF16),
            pltpu.VMEM((NC, S, L), BF16),
            pltpu.VMEM((NC, S, L), BF16),
            pltpu.VMEM((NC, L, S), BF16),
            pltpu.VMEM((NC, L, 3 * D), BF16),
            pltpu.VMEM((D, D), BF16),
            pltpu.VMEM((3 * NC * NC, L, L), BF16),
            pltpu.VMEM((NC * NC, L, L), BF16),
            pltpu.VMEM((3, D, L), F32),
            pltpu.VMEM((8 + S, L), F32),
            pltpu.VMEM((NC, 8, L), F32),
            pltpu.VMEM((NC * NCH, 2 * L, L), BF16),
            pltpu.VMEM((F_ROWS, L), F32),
            pltpu.VMEM((P_ROWS, L), F32),
            pltpu.VMEM((P_ROWS, L), F32),
            pltpu.VMEM((NC, S, L), BF16),
            pltpu.VMEM((NC * S, L), F32),
            pltpu.VMEM((RT * WIN, L), F32),
            pltpu.VMEM((S, D), BF16),
            pltpu.SemaphoreType.DMA((7 * NC + 1,)),
            pltpu.SemaphoreType.DMA((NCH,)),
        ],
        compiler_params=pltpu.CompilerParams(vmem_limit_bytes=110 * 1024 * 1024, flags=({os.environ['FLAG']: True} if 'FLAG' in os.environ else None)),
    )(
        A_q.reshape(S, D), A_k.reshape(S, D), A_v.reshape(S, D),
        A_shift_k.T, A_ssm_k, A_ssm_D, B_wqkv, B_wo, gate_w,
        _FWD, _INV, np.zeros((1,), np.int32),
    )
    return out.reshape(1, S, D)
```

```python
import jax
import jax.numpy as jnp
import numpy as np
from jax import lax
from jax.experimental import pallas as pl
from jax.experimental.pallas import tpu as pltpu

S = 2048
D = 640
NH = 32
DH = D // NH
WIN = 8
DIL = 2
KS = 4
L = 128
NC = D // L
NCH = S // L
NF8 = L // 8
HALO = 16
RT = 256
NRT = S // RT
import os
REDUCE = os.environ.get('REDUCE', 'xlu')
AR = int(os.environ.get('AR', 16))
NT_GROUP = int(os.environ.get('NTG', 1))
RT = int(os.environ.get('RT', 256)); NRT = S // RT
SB = int(os.environ.get('SB', 4))
XF0 = 0
HF0 = XF0 + NC * NCH * 3 * L
XTOK = HF0 + NC * NCH * 3 * L
F_ROWS = XTOK + 8 * NRT
PT = HALO + RT
PTOK = 3 * NC * PT
P_ROWS = PTOK + 8 * NRT
SR = int(os.environ.get('SR', 32)); LAG = int(os.environ.get('LAG', 3)); PRE = float(os.environ.get('PRE', 0.015)); POST = float(os.environ.get('POST', 0.0))
U_PHASE = int(os.environ.get('UP', 13)); U_FIRST = NC * NF8 - (NRT - 3) * U_PHASE
N_IN_SEMS = 3 + 4 * NC + 1 + 4 + 1
_e = lambda n, d: type(d)(os.environ.get(n, d))
A1 = _e('A1', 0.0); A7 = _e('A7', 0.5); T1 = _e('T1', 4); T2 = _e('T2', 11); FR = _e('FR', 128)
F32 = jnp.float32
BF16 = jnp.bfloat16


def _dft_matrices():
    n = np.arange(L)
    k = np.arange(L)
    ang = 2.0 * np.pi * (((4 * k[:, None] + 1) * n[None, :]) % (4 * L)) / (4 * L)
    fwd = np.concatenate([np.cos(ang), -np.sin(ang)], axis=0)
    inv = fwd.reshape(2, NF8, 8, L).transpose(1, 0, 2, 3).reshape(2 * L, L).T / L
    return fwd.astype(BF16), np.ascontiguousarray(inv).astype(BF16)


_FWD, _INV = _dft_matrices()
_SAME_HEAD = (np.arange(L)[:, None] % NH == np.arange(L)[None, :] % NH).astype(BF16)
_NT = (((1,), (1,)), ((), ()))


def _kernel(q_hbm, k_hbm, v_hbm, shift_ref, hk_hbm, ssmd_ref, w_hbm, wo_hbm, gate_ref,
            fwd_ref, inv_ref, zero_ref, out_hbm,
            q_s, k_s, v_s, hk_s, w_s, wo_s, wp_s, wop_s, tmp_s, kf_s, par_s, g_s,
            z_s, f_s, pa_s, pb_s, o_s, b_s, lg_s, out_s, in_sem, out_sem):
    sems = iter(range(N_IN_SEMS))

    def copy(src, dst):
        return pltpu.make_async_copy(src, dst, in_sem.at[next(sems)])

    w_cp = [copy(w_hbm.at[:, pl.ds(p * D, D)], w_s.at[p]) for p in range(3)]
    q_cp = [[copy(q_hbm.at[pl.ds(r0, n), pl.ds(c * L, L)], q_s.at[c, pl.ds(r0, n), :])
             for c in range(NC)]
            for r0, n in ((0, RT), (RT, RT), (2 * RT, RT), (3 * RT, S - 3 * RT))]
    hk_cp = copy(hk_hbm, hk_s)
    kv_cp = [[copy(src.at[pl.ds(h * S // 2, S // 2), :], dst.at[pl.ds(h * S // 2, S // 2), :])
              for src, dst in ((k_hbm, k_s), (v_hbm, v_s))] for h in range(2)]
    wo_cp = copy(wo_hbm, wo_s)
    for cp in ([w_cp[0]] + q_cp[0] + w_cp[1:] + q_cp[1] + [hk_cp] + kv_cp[0] + kv_cp[1]
               + [wo_cp] + q_cp[2] + q_cp[3]):
        cp.start()

    def wait(copies):
        for cp in copies:
            cp.wait()

    taps = shift_ref[...].astype(F32)
    ssmd = ssmd_ref[...].astype(F32).reshape(1, D)
    gate = gate_ref[...].astype(F32).reshape(1, D)
    for c in range(NC):
        par_s[c, pl.ds(0, KS), :] = taps[:, c * L:(c + 1) * L]
        par_s[c, pl.ds(KS, 1), :] = ssmd[:, c * L:(c + 1) * L]
        par_s[c, pl.ds(KS + 1, 1), :] = gate[:, c * L:(c + 1) * L]
    for c in range(NC):
        kf_s[c, pl.ds(0, 8), :] = jnp.zeros((8, L), F32)
    for n in range(NC, 3 * NC):
        pa_s[pl.ds(n * PT, HALO), :] = jnp.zeros((HALO, L), F32)

    def filter_dft(c):
        prev = None
        for m in range(NCH):
            h = lax.dot_general(
                fwd_ref[...], hk_s[c * L:(c + 1) * L, m * L:(m + 1) * L], _NT, preferred_element_type=F32)
            hr, hi = h[:L], h[L:]
            if m == 0:
                hr = hr + par_s[c, pl.ds(KS, 1), :]
                a, b = hr, hi
            else:
                a, b = hr - prev[1], hi + prev[0]
            prev = (hr, hi)
            f_s[pl.ds(HF0 + (c * NCH + m) * 3 * L + 0, L), :] = a
            f_s[pl.ds(HF0 + (c * NCH + m) * 3 * L + L, L), :] = b - a
            f_s[pl.ds(HF0 + (c * NCH + m) * 3 * L + 2 * L, L), :] = a + b
            yield h[L - 8:L]
            yield h[2 * L - 8:]

    def signal_dft(j):
        for c in range(NC):
            rows, cols = pl.ds(j * L, L), slice(c * L, (c + 1) * L)
            k = k_s[rows, cols].astype(F32)
            kf_s[c, pl.ds(8 + j * L, L), :] = k
            ks = k * par_s[c, pl.ds(0, 1), :]
            for t in range(1, KS):
                ks = ks + kf_s[c, pl.ds(8 + j * L - t, L), :] * par_s[c, pl.ds(t, 1), :]
            kv = ks * v_s[rows, cols].astype(F32)
            x = jnp.dot(fwd_ref[...], kv.astype(BF16), preferred_element_type=F32)
            f_s[pl.ds(XF0 + (c * NCH + j) * 3 * L, L), :] = x[:L] + x[L:]
            f_s[pl.ds(XF0 + (c * NCH + j) * 3 * L + L, 2 * L), :] = x
            yield x[2 * L - 8:]

    def head_major_to_dim_major(p):
        return jnp.concatenate([tmp_s[p, pl.ds(d, NH, stride=DH), :] for d in range(DH)], axis=0)

    def permute_wqkv(p):
        for rb in range(NC):
            tmp_s[rb] = w_s[p, rb * L:(rb + 1) * L, :].astype(F32).T
            wt = head_major_to_dim_major(rb).astype(BF16)
            for c in range(NC):
                wp_s[(p * NC + c) * NC + rb] = wt[c * L:(c + 1) * L]

    def permute_wo():
        for c in range(NC):
            tmp_s[c] = wo_s[:, c * L:(c + 1) * L].astype(F32)
            wt = head_major_to_dim_major(c).astype(BF16)
            for rb in range(NC):
                wop_s[c * NC + rb] = wt[rb * L:(rb + 1) * L]

    def spectral(u):
        c, f8 = u // NF8, u % NF8

        def conv(part, i0, acc, sign):
            row = c * NCH * 3 * L + part * L + f8 * 8
            h = {}
            for j in range(i0 + SB):
                x = f_s[pl.ds(pl.multiple_of(XF0 + row + j * 3 * L, 8), 8), :]
                for i in range(max(i0, j), i0 + SB):
                    if i - j not in h:
                        h[i - j] = f_s[pl.ds(pl.multiple_of(HF0 + row + (i - j) * 3 * L, 8), 8), :]
                    p = h[i - j] * x
                    prev = acc[i - i0]
                    acc[i - i0] = p if prev is None else (prev + p if sign > 0 else prev - p)
                yield 2 * (i0 + SB - max(i0, j))

        for i0 in range(0, NCH, SB):
            k1 = [None] * SB
            yield from conv(0, i0, k1, 1)
            zr = list(k1)
            yield from conv(2, i0, zr, -1)
            yield from conv(1, i0, k1, 1)
            for i in range(SB):
                z_s[c * NCH + i0 + i, pl.ds(pl.multiple_of(f8 * 16, 16), 16), :] = jnp.concatenate(
                    [zr[i], k1[i]], axis=0).astype(BF16)
            yield SB

    qscale = float(DH ** -0.5 * np.log2(np.e))

    def attention(r0, src):
        def shifted(base, c, g, w):
            return src[pl.ds((base + c) * PT + HALO + 8 * g - DIL * w, 8), :]

        def scores(g):
            qs = [shifted(0, c, g, 0) for c in range(NC)]
            for w in range(WIN):
                acc = qs[0] * shifted(NC, 0, g, w)
                for c in range(1, NC):
                    acc = acc + qs[c] * shifted(NC, c, g, w)
                acc = acc + pltpu.roll(acc, 2 * NH, 1)
                acc = acc + pltpu.roll(acc, NH, 1)
                if 8 * g < DIL * w:
                    pos = r0 + 8 * g + lax.broadcasted_iota(jnp.int32, (8, L), 0)
                    acc = jnp.where(pos >= DIL * w, acc, -1e9)
                lg_s[pl.ds(8 * (g * WIN + w), 8), :] = acc
                yield 11

        def mix(g):
            logits = [lg_s[pl.ds(8 * (g * WIN + w), 8), :] for w in range(WIN)]
            m = logits[0]
            for w in range(1, WIN):
                m = jnp.maximum(m, logits[w])
            e = [jnp.exp2(l - m) for l in logits]
            den = e[0]
            for w in range(1, WIN):
                den = den + e[w]
            inv = pl.reciprocal(den, approx=True)
            inv = inv * (2.0 - den * inv)
            yield 30
            for c in range(NC):
                acc = e[0] * shifted(2 * NC, c, g, 0)
                for w in range(1, WIN):
                    acc = acc + e[w] * shifted(2 * NC, c, g, w)
                acc = acc * inv
                if g % 2 == 0:
                    half[c] = acc
                else:
                    o_s[c, pl.ds(r0 + 8 * (g - 1), 16), :] = jnp.concatenate(
                        [half[c], acc], axis=0).astype(BF16)
                yield 16

        groups = RT // 8
        half = [None] * NC
        for g in range(groups + LAG):
            if g < groups:
                yield from scores(g)
            if g >= LAG:
                yield from mix(g - LAG)

    def projections(jobs):
        def dot(job, ks):
            lhs_ref, r0, w_ref, n = job[:4]
            lhs = jnp.concatenate([lhs_ref[c, pl.ds(r0, RT), :] for c in ks], axis=1)
            if w_ref is wp_s:
                w = jnp.concatenate([w_ref[n * NC + c] for c in ks], axis=1)
                return lax.dot_general(lhs, w, _NT, preferred_element_type=F32)
            w = jnp.concatenate([w_ref[n * NC + c] for c in ks], axis=0)
            return jnp.dot(lhs, w, preferred_element_type=F32)

        rounds = []
        for g in range(0, len(jobs), 4):
            rounds += [[(job, dot(job, range(NC - 1)))] for job in jobs[g:g + 4]]
            rounds.append([(job, dot(job, [NC - 1])) for job in jobs[g:g + 4]])

        def stores():
            for i, rnd in enumerate(rounds):
                last = i % 5 == 4 or i == len(rounds) - 1
                for r in range(0, RT, SR):
                    for (_, _, _, _, dst, row, scale), y in rnd:
                        rows = pl.ds(row + r, SR)
                        yr = y[r:r + SR]
                        if last:
                            yr = yr + dst[rows, :]
                            yr = yr if scale is None else yr * scale
                        dst[rows, :] = yr
                    yield yr[SR - 8:]

        return stores(), len(rounds) * RT // SR

    def qkv_jobs(r0, dst):
        return [(q_s, r0, wp_s, n, dst, n * PT + HALO, qscale if n < NC else None)
                for n in range(3 * NC)]

    def out_jobs(r0):
        return [(o_s, r0, wop_s, n, b_s, n * S + r0, None) for n in range(NC)]

    def chain(*gens):
        for g in gens:
            yield from g

    def weave(lead, steps, followers):
        done = [0] * len(followers)

        def advance(frac, anchor):
            for i, (gen, work, pace) in enumerate(followers):
                if anchor is not None and done[i] < frac * work:
                    pace(anchor)
                while done[i] < frac * work:
                    done[i] += next(gen)

        advance(PRE / (1 + PRE + POST), None)
        for i, anchor in enumerate(lead):
            advance(min((PRE + (i + 1) / steps) / (1 + PRE + POST), 1.0), anchor)
        advance(1.0, None)

    def gating(r0):
        for r in range(0, RT, 16):
            rows = pl.ds(r0 + r, 16)
            dot = q_s[0, rows, :].astype(F32) * par_s[0, pl.ds(KS + 1, 1), :]
            for c in range(1, NC):
                dot = dot + q_s[c, rows, :].astype(F32) * par_s[c, pl.ds(KS + 1, 1), :]
            g = jax.nn.sigmoid(jnp.sum(dot, axis=-1, keepdims=True))
            g_s[rows, :] = jnp.broadcast_to(g, (16, L))
            yield 1

    def out_copy(i):
        rows = pl.ds(i * L, L)
        return pltpu.make_async_copy(out_s.at[rows, :], out_hbm.at[rows, :], out_sem.at[i])

    def finish(i):
        for c in range(NC):
            y = jnp.dot(inv_ref[...], z_s[c * NCH + i], preferred_element_type=F32)
            for r in range(0, L, FR):
                rows = pl.ds(i * L + r, FR)
                b = b_s[pl.ds(c * S + i * L + r, FR), :]
                a = q_s[c, rows, :].astype(F32) * y[r:r + FR]
                out_s[rows, c * L:(c + 1) * L] = (b + g_s[rows, :] * (a - b)).astype(BF16)
            yield y[L - 8:]

    attn_work = (RT // 8) * (11 * WIN + 30 + 16 * NC)

    def attn_stream(t, src):
        def pace(y):
            src[pl.ds(pl.multiple_of(PTOK + anywhere, 8), 8), :] = y
        return attention(pl.multiple_of(t * RT, RT), src), attn_work, pace

    def spec_stream(u0, n):
        def pace(y):
            f_s[pl.ds(pl.multiple_of(XTOK + anywhere, 8), 8), :] = y
        return chain(*[spectral(u0 + i) for i in range(n)]), n * (3 * NCH * (NCH + 1) + NCH), pace

    def gate_stream(r0):
        def pace(y):
            par_s[NC, pl.ds(pl.multiple_of(anywhere, 8), 8), :] = y
        return gating(r0), RT // 16, pace

    def part(stream, lo, hi):
        gen, work, pace = stream
        return gen, int(work * hi) // 8 * 8 - int(work * lo) // 8 * 8, pace

    def carry_halo(src, dst):
        for n in range(NC, 3 * NC):
            dst[pl.ds(n * PT, HALO), :] = src[pl.ds(n * PT + RT, HALO), :]

    anywhere = zero_ref[0]

    first = qkv_jobs(0, pa_s)
    w_cp[0].wait()
    permute_wqkv(0)
    wait(q_cp[0] + [w_cp[1]])
    permute_wqkv(1)
    weave(*projections(first[:4]), [])
    w_cp[2].wait()
    permute_wqkv(2)
    weave(*projections(first[4:]), [gate_stream(0)])

    wait(q_cp[1])
    carry_halo(pa_s, pb_s)
    weave(*projections(qkv_jobs(RT, pb_s)), [attn_stream(0, pa_s), gate_stream(RT)])

    hk_cp.wait()
    gen, work, pace = attn_stream(1, pb_s)
    shares = [int(work * A1), (work - int(work * A1)) // 2]
    weave(chain(*[filter_dft(c) for c in range(NC)]), 2 * NC * NCH, [(gen, shares[0], pace)])

    for h in range(2):
        wait(kv_cp[h])
        weave(chain(*[signal_dft(j) for j in range(h * NCH // 2, (h + 1) * NCH // 2)]),
              NC * NCH // 2, [(gen, shares[1] - 40, pace)])
    for _ in gen:
        pass

    wait([wo_cp] + q_cp[2])
    permute_wo()
    carry_halo(pb_s, pa_s)
    weave(*projections(qkv_jobs(2 * RT, pa_s) + out_jobs(0)),
          [spec_stream(0, U_FIRST), gate_stream(2 * RT)])
    wait(q_cp[3])

    def phase(t, cur, nxt):
        row = lambda i: pl.multiple_of(i * RT, RT)
        carry_halo(cur, nxt)
        weave(*projections(out_jobs(row(t - 1)) + qkv_jobs(row(t + 1), nxt)),
              [attn_stream(t, cur), spec_stream(U_FIRST + (t - 2) * U_PHASE, U_PHASE),
               gate_stream(row(t + 1))])

    @pl.loop(0, (NRT - 2) // 2)
    def _(i):
        phase(2 * i + 2, pa_s, pb_s)

        @pl.when(i < (NRT - 2) // 2 - 1)
        def _():
            phase(2 * i + 3, pb_s, pa_s)

    def tail(chunks, jobs, followers):
        lead, steps = projections(jobs) if jobs else ((), 0)
        weave(chain(lead, *[finish(i) for i in chunks]), steps + len(chunks) * NC, followers)

    gen, work, pace = attn_stream(NRT - 1, pb_s)
    tail(range(0, T1), out_jobs(S - 2 * RT), [(gen, int(work * A7), pace)])
    for i in range(0, T1):
        out_copy(i).start()
    tail(range(T1, T2), None, [(gen, work - int(work * A7) - 40, pace)])
    for _ in gen:
        pass
    for i in range(T1, T2):
        out_copy(i).start()
    tail(range(T2, NCH - 2), out_jobs(S - RT), [])
    for i in range(T2, NCH - 2):
        out_copy(i).start()
    for i in range(NCH - 2, NCH):
        tail([i], None, [])
        out_copy(i).start()
    for i in range(NCH):
        out_copy(i).wait()


@jax.jit
def pallas_gated_mix__ssm_conv_h3__sliding_local_dilated__prompt_kernel(
    A_q: jax.Array,
    A_k: jax.Array,
    A_v: jax.Array,
    A_shift_k: jax.Array,
    A_ssm_k: jax.Array,
    A_ssm_D: jax.Array,
    B_x: jax.Array,
    B_wqkv: jax.Array,
    B_wo: jax.Array,
    gate_w: jax.Array,
):
    del B_x
    hbm = pl.BlockSpec(memory_space=pl.ANY)
    vmem = pl.BlockSpec(memory_space=pltpu.VMEM)
    smem = pl.BlockSpec(memory_space=pltpu.SMEM)
    out = pl.pallas_call(
        _kernel,
        out_shape=jax.ShapeDtypeStruct((S, D), BF16),
        in_specs=[hbm, hbm, hbm, vmem, hbm, vmem, hbm, hbm, vmem, vmem, vmem, smem],
        out_specs=hbm,
        scratch_shapes=[
            pltpu.VMEM((NC, S, L), BF16),
            pltpu.VMEM((S, D), BF16),
            pltpu.VMEM((S, D), BF16),
            pltpu.VMEM((D, S), BF16),
            pltpu.VMEM((3, D, D), BF16),
            pltpu.VMEM((D, D), BF16),
            pltpu.VMEM((3 * NC * NC, L, L), BF16),
            pltpu.VMEM((NC * NC, L, L), BF16),
            pltpu.VMEM((NC, D, L), F32),
            pltpu.VMEM((NC, 8 + S, L), F32),
            pltpu.VMEM((NC + 1, 8, L), F32),
            pltpu.VMEM((S, L), F32),
            pltpu.VMEM((NC * NCH, 2 * L, L), BF16),
            pltpu.VMEM((F_ROWS, L), F32),
            pltpu.VMEM((P_ROWS, L), F32),
            pltpu.VMEM((P_ROWS, L), F32),
            pltpu.VMEM((NC, S, L), BF16),
            pltpu.VMEM((NC * S, L), F32),
            pltpu.VMEM((RT * WIN, L), F32),
            pltpu.VMEM((S, D), BF16),
            pltpu.SemaphoreType.DMA((N_IN_SEMS,)),
            pltpu.SemaphoreType.DMA((NCH,)),
        ],
        compiler_params=pltpu.CompilerParams(vmem_limit_bytes=110 * 1024 * 1024, flags=({os.environ['FLAG']: True} if 'FLAG' in os.environ else None)),
    )(
        A_q.reshape(S, D), A_k.reshape(S, D), A_v.reshape(S, D),
        A_shift_k.T, A_ssm_k, A_ssm_D, B_wqkv, B_wo, gate_w,
        _FWD, _INV, np.zeros((1,), np.int32),
    )
    return out.reshape(1, S, D)
```

```python
import jax
import jax.numpy as jnp
import numpy as np
from jax import lax
from jax.experimental import pallas as pl
from jax.experimental.pallas import tpu as pltpu

S = 2048
D = 640
NH = 32
DH = D // NH
WIN = 8
DIL = 2
KS = 4
L = 128
NC = D // L
NCH = S // L
NF8 = L // 8
HALO = 16
RT = 256
NRT = S // RT
import os
REDUCE = os.environ.get('REDUCE', 'xlu')
AR = int(os.environ.get('AR', 16))
NT_GROUP = int(os.environ.get('NTG', 1))
RT = int(os.environ.get('RT', 256)); NRT = S // RT
SB = int(os.environ.get('SB', 8))
PADF = int(os.environ.get('PADF', 16)); PADB = int(os.environ.get('PADB', 16)); PADW = int(os.environ.get('PADW', 16)); PADP = int(os.environ.get('PADP', 8))
PS = L + int(os.environ.get('PADS', 0))
FS = 3 * PS + PADF
XF0 = 0
HF0 = XF0 + NC * NCH * FS + int(os.environ.get('PADH', 8))
XTOK = HF0 + NC * NCH * FS
F_ROWS = XTOK + 8 * NRT
PT = HALO + RT + PADP
BS = S + PADP
PTOK = 3 * NC * PT
P_ROWS = PTOK + 8 * NRT
SR = int(os.environ.get('SR', 32)); LAG = int(os.environ.get('LAG', 3)); PRE = float(os.environ.get('PRE', 0.015)); POST = float(os.environ.get('POST', 0.0))
U_PHASE = int(os.environ.get('UP', 13)); U_FIRST = NC * NF8 - (NRT - 3) * U_PHASE
N_IN_SEMS = 3 + 4 * NC + 1 + 4 + 1 + 6
_e = lambda n, d: type(d)(os.environ.get(n, d))
A1 = _e('A1', 1.0); A7 = _e('A7', 0.5); T1 = _e('T1', 4); T2 = _e('T2', 11); FR = _e('FR', 128)
F32 = jnp.float32
U32 = jnp.uint32
BF16 = jnp.bfloat16


def _dft_matrices():
    n = np.arange(L)
    k = np.arange(L)
    ang = 2.0 * np.pi * (((4 * k[:, None] + 1) * n[None, :]) % (4 * L)) / (4 * L)
    fwd = np.concatenate([np.cos(ang), -np.sin(ang)], axis=0)
    inv = fwd.reshape(2, NF8, 8, L).transpose(1, 0, 2, 3).reshape(2 * L, L).T / L
    return fwd.astype(BF16), np.ascontiguousarray(inv).astype(BF16)


_FWD, _INV = _dft_matrices()
_SAME_HEAD = (np.arange(L)[:, None] % NH == np.arange(L)[None, :] % NH).astype(BF16)
_NT = (((1,), (1,)), ((), ()))


def _kernel(q_hbm, k_hbm, v_hbm, shift_hbm, hk_hbm, ssmd_hbm, w_hbm, wo_hbm, gate_hbm,
            fwd_hbm, inv_hbm, zero_hbm, out_hbm,
            shift_ref, ssmd_ref, gate_ref, fwd_ref, inv_ref, zero_ref,
            q_s, k_s, v_s, hk_s, w_s, wo_s, wp_s, wop_s, tmp_s, kf_s, par_s, g_s,
            z_s, f_s, pa_s, pb_s, o_s, b_s, lg_s, out_s, in_sem, out_sem):
    sems = iter(range(N_IN_SEMS))

    def copy(src, dst):
        return pltpu.make_async_copy(src, dst, in_sem.at[next(sems)])

    w_cp = [copy(w_hbm.at[:, pl.ds(p * D, D)], w_s.at[p]) for p in range(3)]
    q_cp = [[copy(q_hbm.at[pl.ds(r0, n), pl.ds(c * L, L)], q_s.at[c, pl.ds(r0, n), :])
             for c in range(NC)]
            for r0, n in ((0, RT), (RT, RT), (2 * RT, RT), (3 * RT, S - 3 * RT))]
    hk_cp = copy(hk_hbm, hk_s)
    kv_cp = [[copy(src.at[pl.ds(h * S // 2, S // 2), :], dst.at[pl.ds(h * S // 2, S // 2), :])
              for src, dst in ((k_hbm, k_s), (v_hbm, v_s))] for h in range(2)]
    wo_cp = copy(wo_hbm, wo_s)
    small_cp = [copy(zero_hbm, zero_ref), copy(shift_hbm, shift_ref), copy(ssmd_hbm, ssmd_ref),
                copy(gate_hbm, gate_ref)]
    dft_cp = [copy(fwd_hbm, fwd_ref), copy(inv_hbm, inv_ref)]
    for cp in (small_cp + [w_cp[0]] + q_cp[0] + w_cp[1:] + q_cp[1] + dft_cp + [hk_cp] + kv_cp[0] + kv_cp[1]
               + [wo_cp] + q_cp[2] + q_cp[3]):
        cp.start()

    def wait(copies):
        for cp in copies:
            cp.wait()

    wait(small_cp)
    taps = shift_ref[...].astype(F32)
    ssmd = ssmd_ref[...].astype(F32).reshape(1, D)
    gate = gate_ref[...].astype(F32).reshape(1, D)
    for c in range(NC):
        par_s[c, pl.ds(0, KS), :] = taps[:, c * L:(c + 1) * L]
        par_s[c, pl.ds(KS, 1), :] = ssmd[:, c * L:(c + 1) * L]
        par_s[c, pl.ds(KS + 1, 1), :] = gate[:, c * L:(c + 1) * L]
    for c in range(NC):
        kf_s[c, pl.ds(0, 8), :] = jnp.zeros((8, L), F32)
    for n in range(NC, 3 * NC):
        pa_s[pl.ds(n * PT, HALO), :] = jnp.zeros((HALO, L), F32)

    def filter_dft(c):
        prev = None
        for m in range(NCH):
            h = lax.dot_general(
                fwd_ref[...], hk_s[c * L:(c + 1) * L, m * L:(m + 1) * L], _NT, preferred_element_type=F32)
            hr, hi = h[:L], h[L:]
            if m == 0:
                hr = hr + par_s[c, pl.ds(KS, 1), :]
                a, b = hr, hi
            else:
                a, b = hr - prev[1], hi + prev[0]
            prev = (hr, hi)
            f_s[pl.ds(HF0 + (c * NCH + m) * FS + 0, L), :] = a
            f_s[pl.ds(HF0 + (c * NCH + m) * FS + PS, L), :] = b - a
            f_s[pl.ds(HF0 + (c * NCH + m) * FS + 2 * PS, L), :] = a + b
            yield h[L - 8:L]
            yield h[2 * L - 8:]

    def signal_dft(j):
        for c in range(NC):
            rows, cols = pl.ds(j * L, L), slice(c * L, (c + 1) * L)
            k = k_s[rows, cols].astype(F32)
            kf_s[c, pl.ds(8 + j * L, L), :] = k
            ks = k * par_s[c, pl.ds(0, 1), :]
            for t in range(1, KS):
                ks = ks + kf_s[c, pl.ds(8 + j * L - t, L), :] * par_s[c, pl.ds(t, 1), :]
            kv = ks * v_s[rows, cols].astype(F32)
            x = jnp.dot(fwd_ref[...], kv.astype(BF16), preferred_element_type=F32)
            f_s[pl.ds(XF0 + (c * NCH + j) * FS, L), :] = x[:L] + x[L:]
            f_s[pl.ds(XF0 + (c * NCH + j) * FS + PS, L), :] = x[:L]
            f_s[pl.ds(XF0 + (c * NCH + j) * FS + 2 * PS, L), :] = x[L:]
            yield x[2 * L - 8:]

    def head_major_to_dim_major(p):
        return jnp.concatenate([tmp_s[p, pl.ds(d, NH, stride=DH), :] for d in range(DH)], axis=0)

    def permute_wqkv(p):
        for rb in range(NC):
            tmp_s[rb] = w_s[p, rb * L:(rb + 1) * L, :].astype(F32).T
            wt = head_major_to_dim_major(rb).astype(BF16)
            for c in range(NC):
                wp_s[(p * NC + c) * NC + rb] = pltpu.bitcast(wt[c * L:(c + 1) * L], U32)

    def permute_wo():
        for c in range(NC):
            tmp_s[c] = wo_s[:, c * L:(c + 1) * L].astype(F32)
            wt = head_major_to_dim_major(c).astype(BF16)
            for rb in range(NC):
                wop_s[c * NC + rb] = pltpu.bitcast(wt[rb * L:(rb + 1) * L], U32)

    def spectral(u):
        c, f8 = u // NF8, u % NF8

        def conv(part, i0, acc, sign):
            row = c * NCH * FS + part * PS + f8 * 8
            h = {}
            for j in range(i0 + SB):
                x = f_s[pl.ds(pl.multiple_of(XF0 + row + j * FS, 8), 8), :]
                for i in range(max(i0, j), i0 + SB):
                    if i - j not in h:
                        h[i - j] = f_s[pl.ds(pl.multiple_of(HF0 + row + (i - j) * FS, 8), 8), :]
                    p = h[i - j] * x
                    prev = acc[i - i0]
                    acc[i - i0] = p if prev is None else (prev + p if sign > 0 else prev - p)
                yield 2 * (i0 + SB - max(i0, j))

        for i0 in range(0, NCH, SB):
            k1 = [None] * SB
            yield from conv(0, i0, k1, 1)
            zr = list(k1)
            yield from conv(2, i0, zr, -1)
            yield from conv(1, i0, k1, 1)
            for i in range(SB):
                z = jnp.concatenate([zr[i], k1[i]], axis=0).astype(BF16)
                z_s[c * NCH + i0 + i, pl.ds(pl.multiple_of(f8 * 8, 8), 8), :] = pltpu.bitcast(z, U32)
            yield SB

    qscale = float(DH ** -0.5 * np.log2(np.e))

    def attention(r0, src):
        def shifted(base, c, g, w):
            return src[pl.ds((base + c) * PT + HALO + 8 * g - DIL * w, 8), :]

        def scores(g):
            qs = [shifted(0, c, g, 0) for c in range(NC)]
            for w in range(WIN):
                acc = qs[0] * shifted(NC, 0, g, w)
                for c in range(1, NC):
                    acc = acc + qs[c] * shifted(NC, c, g, w)
                acc = acc + pltpu.roll(acc, 2 * NH, 1)
                acc = acc + pltpu.roll(acc, NH, 1)
                if 8 * g < DIL * w:
                    pos = r0 + 8 * g + lax.broadcasted_iota(jnp.int32, (8, L), 0)
                    acc = jnp.where(pos >= DIL * w, acc, -1e9)
                lg_s[pl.ds(8 * (g * WIN + w), 8), :] = acc
                yield 11

        def mix(g):
            logits = [lg_s[pl.ds(8 * (g * WIN + w), 8), :] for w in range(WIN)]
            m = logits[0]
            for w in range(1, WIN):
                m = jnp.maximum(m, logits[w])
            e = [jnp.exp2(l - m) for l in logits]
            den = e[0]
            for w in range(1, WIN):
                den = den + e[w]
            inv = pl.reciprocal(den, approx=True)
            inv = inv * (2.0 - den * inv)
            yield 30
            for c in range(NC):
                acc = e[0] * shifted(2 * NC, c, g, 0)
                for w in range(1, WIN):
                    acc = acc + e[w] * shifted(2 * NC, c, g, w)
                acc = acc * inv
                if g % 2 == 0:
                    half[c] = acc
                else:
                    o_s[c, pl.ds(r0 + 8 * (g - 1), 16), :] = jnp.concatenate(
                        [half[c], acc], axis=0).astype(BF16)
                yield 16

        groups = RT // 8
        half = [None] * NC
        for g in range(groups + LAG):
            if g < groups:
                yield from scores(g)
            if g >= LAG:
                yield from mix(g - LAG)

    def projections(jobs):
        def dot(job, ks):
            lhs_ref, r0, w_ref, n = job[:4]
            lhs = jnp.concatenate([lhs_ref[c, pl.ds(r0, RT), :] for c in ks], axis=1)
            if w_ref is wp_s:
                w = jnp.concatenate([pltpu.bitcast(w_ref[n * NC + c], BF16) for c in ks], axis=1)
                return lax.dot_general(lhs, w, _NT, preferred_element_type=F32)
            w = jnp.concatenate([pltpu.bitcast(w_ref[n * NC + c], BF16) for c in ks], axis=0)
            return jnp.dot(lhs, w, preferred_element_type=F32)

        rounds = []
        for g in range(0, len(jobs), 4):
            rounds += [[(job, dot(job, range(NC - 1)))] for job in jobs[g:g + 4]]
            rounds.append([(job, dot(job, [NC - 1])) for job in jobs[g:g + 4]])

        def stores():
            for i, rnd in enumerate(rounds):
                last = i % 5 == 4 or i == len(rounds) - 1
                for r in range(0, RT, SR):
                    for (_, _, _, _, dst, row, scale), y in rnd:
                        rows = pl.ds(row + r, SR)
                        yr = y[r:r + SR]
                        if last:
                            yr = yr + dst[rows, :]
                            yr = yr if scale is None else yr * scale
                        dst[rows, :] = yr
                    yield yr[SR - 8:]

        return stores(), len(rounds) * RT // SR

    def qkv_jobs(r0, dst):
        return [(q_s, r0, wp_s, n, dst, n * PT + HALO, qscale if n < NC else None)
                for n in range(3 * NC)]

    def out_jobs(r0):
        return [(o_s, r0, wop_s, n, b_s, n * BS + r0, None) for n in range(NC)]

    def chain(*gens):
        for g in gens:
            yield from g

    def weave(lead, steps, followers):
        done = [0] * len(followers)

        def advance(frac, anchor):
            for i, (gen, work, pace) in enumerate(followers):
                if anchor is not None and done[i] < frac * work:
                    pace(anchor)
                while done[i] < frac * work:
                    done[i] += next(gen)

        advance(PRE / (1 + PRE + POST), None)
        for i, anchor in enumerate(lead):
            advance(min((PRE + (i + 1) / steps) / (1 + PRE + POST), 1.0), anchor)
        advance(1.0, None)

    def gating(r0):
        for r in range(0, RT, 16):
            rows = pl.ds(r0 + r, 16)
            dot = q_s[0, rows, :].astype(F32) * par_s[0, pl.ds(KS + 1, 1), :]
            for c in range(1, NC):
                dot = dot + q_s[c, rows, :].astype(F32) * par_s[c, pl.ds(KS + 1, 1), :]
            g = jax.nn.sigmoid(jnp.sum(dot, axis=-1, keepdims=True))
            g_s[rows, :] = jnp.broadcast_to(g, (16, L))
            yield 1

    def out_copy(i):
        rows = pl.ds(i * L, L)
        return pltpu.make_async_copy(out_s.at[rows, :], out_hbm.at[rows, :], out_sem.at[i])

    def finish(i):
        for c in range(NC):
            y = jnp.dot(inv_ref[...], pltpu.bitcast(z_s[c * NCH + i, pl.ds(0, L), :], BF16),
                        preferred_element_type=F32)
            for r in range(0, L, FR):
                rows = pl.ds(i * L + r, FR)
                b = b_s[pl.ds(c * BS + i * L + r, FR), :]
                a = q_s[c, rows, :].astype(F32) * y[r:r + FR]
                out_s[rows, c * L:(c + 1) * L] = (b + g_s[rows, :] * (a - b)).astype(BF16)
            yield y[L - 8:]

    attn_work = (RT // 8) * (11 * WIN + 30 + 16 * NC)

    def attn_stream(t, src):
        def pace(y):
            src[pl.ds(pl.multiple_of(PTOK + anywhere, 8), 8), :] = y
        return attention(pl.multiple_of(t * RT, RT), src), attn_work, pace

    def spec_stream(u0, n):
        def pace(y):
            f_s[pl.ds(pl.multiple_of(XTOK + anywhere, 8), 8), :] = y
        return chain(*[spectral(u0 + i) for i in range(n)]), n * (3 * NCH * (NCH + 1) + NCH), pace

    def gate_stream(r0):
        def pace(y):
            par_s[NC, pl.ds(pl.multiple_of(anywhere, 8), 8), :] = y
        return gating(r0), RT // 16, pace

    def part(stream, lo, hi):
        gen, work, pace = stream
        return gen, int(work * hi) // 8 * 8 - int(work * lo) // 8 * 8, pace

    def carry_halo(src, dst):
        for n in range(NC, 3 * NC):
            dst[pl.ds(n * PT, HALO), :] = src[pl.ds(n * PT + RT, HALO), :]

    anywhere = zero_ref[0]

    first = qkv_jobs(0, pa_s)
    w_cp[0].wait()
    permute_wqkv(0)
    wait(q_cp[0])
    weave(*projections(first[:4]), [])
    w_cp[1].wait()
    permute_wqkv(1)
    weave(*projections(first[4:7]), [])
    w_cp[2].wait()
    permute_wqkv(2)
    weave(*projections(first[7:]), [gate_stream(0)])

    wait(q_cp[1])
    carry_halo(pa_s, pb_s)
    weave(*projections(qkv_jobs(RT, pb_s)), [attn_stream(0, pa_s), gate_stream(RT)])

    wait(dft_cp + [hk_cp])
    gen, work, pace = attn_stream(1, pb_s)
    shares = [int(work * A1), (work - int(work * A1)) // 2]
    weave(chain(*[filter_dft(c) for c in range(NC)]), 2 * NC * NCH, [(gen, shares[0], pace)])

    for h in range(2):
        wait(kv_cp[h])
        weave(chain(*[signal_dft(j) for j in range(h * NCH // 2, (h + 1) * NCH // 2)]),
              NC * NCH // 2, [(gen, shares[1] - 40, pace)])
    for _ in gen:
        pass

    wait([wo_cp] + q_cp[2])
    permute_wo()
    carry_halo(pb_s, pa_s)
    weave(*projections(qkv_jobs(2 * RT, pa_s) + out_jobs(0)),
          [spec_stream(0, U_FIRST), gate_stream(2 * RT)])
    wait(q_cp[3])

    def phase(t, cur, nxt):
        row = lambda i: pl.multiple_of(i * RT, RT)
        carry_halo(cur, nxt)
        weave(*projections(out_jobs(row(t - 1)) + qkv_jobs(row(t + 1), nxt)),
              [attn_stream(t, cur), spec_stream(U_FIRST + (t - 2) * U_PHASE, U_PHASE),
               gate_stream(row(t + 1))])

    @pl.loop(0, (NRT - 2) // 2)
    def _(i):
        phase(2 * i + 2, pa_s, pb_s)

        @pl.when(i < (NRT - 2) // 2 - 1)
        def _():
            phase(2 * i + 3, pb_s, pa_s)

    def tail(chunks, jobs, followers):
        lead, steps = projections(jobs) if jobs else ((), 0)
        weave(chain(lead, *[finish(i) for i in chunks]), steps + len(chunks) * NC, followers)

    gen, work, pace = attn_stream(NRT - 1, pb_s)
    tail(range(0, T1), out_jobs(S - 2 * RT), [(gen, int(work * A7), pace)])
    for i in range(0, T1):
        out_copy(i).start()
    tail(range(T1, T2), None, [(gen, work - int(work * A7) - 40, pace)])
    for _ in gen:
        pass
    for i in range(T1, T2):
        out_copy(i).start()
    tail(range(T2, NCH - 2), out_jobs(S - RT), [])
    for i in range(T2, NCH - 2):
        out_copy(i).start()
    for i in range(NCH - 2, NCH):
        tail([i], None, [])
        out_copy(i).start()
    for i in range(NCH):
        out_copy(i).wait()


@jax.jit
def pallas_gated_mix__ssm_conv_h3__sliding_local_dilated__prompt_kernel(
    A_q: jax.Array,
    A_k: jax.Array,
    A_v: jax.Array,
    A_shift_k: jax.Array,
    A_ssm_k: jax.Array,
    A_ssm_D: jax.Array,
    B_x: jax.Array,
    B_wqkv: jax.Array,
    B_wo: jax.Array,
    gate_w: jax.Array,
):
    del B_x
    hbm = pl.BlockSpec(memory_space=pl.ANY)
    out = pl.pallas_call(
        _kernel,
        out_shape=jax.ShapeDtypeStruct((S, D), BF16),
        in_specs=[hbm] * 12,
        out_specs=hbm,
        scratch_shapes=[
            pltpu.VMEM((KS, D), BF16),
            pltpu.VMEM((D,), BF16),
            pltpu.VMEM((D,), BF16),
            pltpu.VMEM((2 * L, L), BF16),
            pltpu.VMEM((L, 2 * L), BF16),
            pltpu.SMEM((1,), jnp.int32),
            pltpu.VMEM((NC, S + PADB, L), BF16),
            pltpu.VMEM((S, D), BF16),
            pltpu.VMEM((S, D), BF16),
            pltpu.VMEM((D, S), BF16),
            pltpu.VMEM((3, D, D), BF16),
            pltpu.VMEM((D, D), BF16),
            pltpu.VMEM((3 * NC * NC, L // 2, L), U32),
            pltpu.VMEM((NC * NC, L // 2, L), U32),
            pltpu.VMEM((NC, D, L), F32),
            pltpu.VMEM((NC, 8 + S, L), F32),
            pltpu.VMEM((NC + 1, 8, L), F32),
            pltpu.VMEM((S, L), F32),
            pltpu.VMEM((NC * NCH, L + 8, L), U32),
            pltpu.VMEM((F_ROWS, L), F32),
            pltpu.VMEM((P_ROWS, L), F32),
            pltpu.VMEM((P_ROWS, L), F32),
            pltpu.VMEM((NC, S + PADB, L), BF16),
            pltpu.VMEM((NC * BS, L), F32),
            pltpu.VMEM((RT * WIN, L), F32),
            pltpu.VMEM((S, D), BF16),
            pltpu.SemaphoreType.DMA((N_IN_SEMS,)),
            pltpu.SemaphoreType.DMA((NCH,)),
        ],
        compiler_params=pltpu.CompilerParams(vmem_limit_bytes=110 * 1024 * 1024, flags=({os.environ['FLAG']: True} if 'FLAG' in os.environ else None)),
    )(
        A_q.reshape(S, D), A_k.reshape(S, D), A_v.reshape(S, D),
        A_shift_k.T, A_ssm_k, A_ssm_D, B_wqkv, B_wo, gate_w,
        _FWD, _INV, np.zeros((1,), np.int32),
    )
    return out.reshape(1, S, D)
```

```python
import jax
import jax.numpy as jnp
import numpy as np
from jax import lax
from jax.experimental import pallas as pl
from jax.experimental.pallas import tpu as pltpu

S = 2048
D = 640
NH = 32
DH = D // NH
WIN = 8
DIL = 2
KS = 4
L = 128
NC = D // L
NCH = S // L
NF8 = L // 8
HALO = 16
RT = 256
NRT = S // RT
import os
REDUCE = os.environ.get('REDUCE', 'xlu')
AR = int(os.environ.get('AR', 16))
NT_GROUP = int(os.environ.get('NTG', 1))
RT = int(os.environ.get('RT', 256)); NRT = S // RT
SB = int(os.environ.get('SB', 8))
PADF = int(os.environ.get('PADF', 16)); PADB = int(os.environ.get('PADB', 16)); PADW = int(os.environ.get('PADW', 16)); PADP = int(os.environ.get('PADP', 8))
PS = L + int(os.environ.get('PADS', 0))
FS = 3 * PS + PADF
XF0 = 0
HF0 = XF0 + NC * NCH * FS + int(os.environ.get('PADH', 8))
XTOK = HF0 + NC * NCH * FS
F_ROWS = XTOK + 8 * NRT
PT = HALO + RT + PADP
BS = S + PADP
PTOK = 3 * NC * PT
P_ROWS = PTOK + 8 * NRT
SR = int(os.environ.get('SR', 32)); LAG = int(os.environ.get('LAG', 3)); PRE = float(os.environ.get('PRE', 0.03)); POST = float(os.environ.get('POST', 0.0))
U_PHASE = int(os.environ.get('UP', 13)); U_FIRST = NC * NF8 - (NRT - 3) * U_PHASE
KV_SPLIT = [int(x) for x in os.environ.get('KV', '0,8,16').split(',')]
N_IN_SEMS = 3 + 4 * NC + 1 + 2 * (len(KV_SPLIT) - 1) + 1 + 6
_e = lambda n, d: type(d)(os.environ.get(n, d))
A1 = _e('A1', 0.0); A7 = _e('A7', 0.5); T1 = _e('T1', 4); T2 = _e('T2', 11); FR = _e('FR', 128)
F32 = jnp.float32
U32 = jnp.uint32
BLOCKS = [int(x) for x in _e('BL', '0,4,8,12,16').split(',')]; TANH = _e('TANH', 1); LATE = _e('LATE', 0); GT = _e('GT', 0)
BF16 = jnp.bfloat16


def _dft_matrices():
    n = np.arange(L)
    k = np.arange(L)
    ang = 2.0 * np.pi * (((4 * k[:, None] + 1) * n[None, :]) % (4 * L)) / (4 * L)
    fwd = np.concatenate([np.cos(ang), -np.sin(ang)], axis=0)
    inv = fwd.reshape(2, NF8, 8, L).transpose(1, 0, 2, 3).reshape(2 * L, L).T / L
    return fwd.astype(BF16), np.ascontiguousarray(inv).astype(BF16)


_FWD, _INV = _dft_matrices()
_SAME_HEAD = (np.arange(L)[:, None] % NH == np.arange(L)[None, :] % NH).astype(BF16)
_NT = (((1,), (1,)), ((), ()))


def _kernel(q_hbm, k_hbm, v_hbm, shift_hbm, hk_hbm, ssmd_hbm, w_hbm, wo_hbm, gate_hbm,
            fwd_hbm, inv_hbm, zero_hbm, out_hbm,
            shift_ref, ssmd_ref, gate_ref, fwd_ref, inv_ref, zero_ref,
            q_s, k_s, v_s, hk_s, w_s, wo_s, wp_s, wop_s, tmp_s, kf_s, par_s, g_s,
            z_s, f_s, pa_s, pb_s, o_s, b_s, lg_s, out_s, in_sem, out_sem):
    sems = iter(range(N_IN_SEMS))

    def copy(src, dst):
        return pltpu.make_async_copy(src, dst, in_sem.at[next(sems)])

    w_cp = [copy(w_hbm.at[:, pl.ds(p * D, D)], w_s.at[p]) for p in range(3)]
    q_cp = [[copy(q_hbm.at[pl.ds(r0, n), pl.ds(c * L, L)], q_s.at[c, pl.ds(r0, n), :])
             for c in range(NC)]
            for r0, n in ((0, RT), (RT, RT), (2 * RT, RT), (3 * RT, S - 3 * RT))]
    hk_cp = copy(hk_hbm, hk_s)
    kv_cp = [[copy(src.at[pl.ds(j0 * L, (j1 - j0) * L), :], dst.at[pl.ds(j0 * L, (j1 - j0) * L), :])
              for src, dst in ((k_hbm, k_s), (v_hbm, v_s))]
             for j0, j1 in zip(KV_SPLIT[:-1], KV_SPLIT[1:])]
    wo_cp = copy(wo_hbm, wo_s)
    small_cp = [copy(zero_hbm, zero_ref), copy(shift_hbm, shift_ref), copy(ssmd_hbm, ssmd_ref),
                copy(gate_hbm, gate_ref)]
    dft_cp = [copy(fwd_hbm, fwd_ref), copy(inv_hbm, inv_ref)]
    for cp in (small_cp + [w_cp[0]] + q_cp[0] + w_cp[1:] + q_cp[1] + dft_cp + [hk_cp] + sum(kv_cp, [])
               + [wo_cp] + q_cp[2] + q_cp[3]):
        cp.start()

    def wait(copies):
        for cp in copies:
            cp.wait()

    wait(small_cp)
    taps = shift_ref[...].astype(F32)
    ssmd = ssmd_ref[...].astype(F32).reshape(1, D)
    gate = gate_ref[...].astype(F32).reshape(1, D)
    for c in range(NC):
        par_s[c, pl.ds(0, KS), :] = taps[:, c * L:(c + 1) * L]
        par_s[c, pl.ds(KS, 1), :] = ssmd[:, c * L:(c + 1) * L]
        par_s[c, pl.ds(KS + 1, 1), :] = gate[:, c * L:(c + 1) * L]
    for c in range(NC):
        kf_s[c, pl.ds(0, 8), :] = jnp.zeros((8, L), F32)
    for n in range(NC, 3 * NC):
        pa_s[pl.ds(n * PT, HALO), :] = jnp.zeros((HALO, L), F32)

    def filter_dft(c):
        prev = None
        for m in range(NCH):
            h = lax.dot_general(
                fwd_ref[...], hk_s[c * L:(c + 1) * L, m * L:(m + 1) * L], _NT, preferred_element_type=F32)
            hr, hi = h[:L], h[L:]
            if m == 0:
                hr = hr + par_s[c, pl.ds(KS, 1), :]
                a, b = hr, hi
            else:
                a, b = hr - prev[1], hi + prev[0]
            prev = (hr, hi)
            f_s[pl.ds(HF0 + (c * NCH + m) * FS + 0, L), :] = a
            f_s[pl.ds(HF0 + (c * NCH + m) * FS + PS, L), :] = b - a
            f_s[pl.ds(HF0 + (c * NCH + m) * FS + 2 * PS, L), :] = a + b
            yield h[L - 8:L]
            yield h[2 * L - 8:]

    def signal_dft(j):
        for c in range(NC):
            rows, cols = pl.ds(j * L, L), slice(c * L, (c + 1) * L)
            k = k_s[rows, cols].astype(F32)
            kf_s[c, pl.ds(8 + j * L, L), :] = k
            ks = k * par_s[c, pl.ds(0, 1), :]
            for t in range(1, KS):
                ks = ks + kf_s[c, pl.ds(8 + j * L - t, L), :] * par_s[c, pl.ds(t, 1), :]
            kv = ks * v_s[rows, cols].astype(F32)
            x = jnp.dot(fwd_ref[...], kv.astype(BF16), preferred_element_type=F32)
            f_s[pl.ds(XF0 + (c * NCH + j) * FS, L), :] = x[:L] + x[L:]
            f_s[pl.ds(XF0 + (c * NCH + j) * FS + PS, L), :] = x[:L]
            f_s[pl.ds(XF0 + (c * NCH + j) * FS + 2 * PS, L), :] = x[L:]
            yield x[2 * L - 8:]

    def head_major_to_dim_major(p):
        return jnp.concatenate([tmp_s[p, pl.ds(d, NH, stride=DH), :] for d in range(DH)], axis=0)

    def permute_wqkv(p):
        for rb in range(NC):
            tmp_s[rb] = w_s[p, rb * L:(rb + 1) * L, :].astype(F32).T
            wt = head_major_to_dim_major(rb).astype(BF16)
            for c in range(NC):
                wp_s[(p * NC + c) * NC + rb] = pltpu.bitcast(wt[c * L:(c + 1) * L], U32)

    def permute_wo():
        for c in range(NC):
            tmp_s[c] = wo_s[:, c * L:(c + 1) * L].astype(F32)
            wt = head_major_to_dim_major(c).astype(BF16)
            for rb in range(NC):
                wop_s[c * NC + rb] = pltpu.bitcast(wt[rb * L:(rb + 1) * L], U32)

    def spectral(u):
        c, f8 = u // NF8, u % NF8

        def conv(part, i0, i1, acc, sign):
            row = c * NCH * FS + part * PS + f8 * 8
            h = {}
            for j in range(i1):
                x = f_s[pl.ds(pl.multiple_of(XF0 + row + j * FS, 8), 8), :]
                for i in range(max(i0, j), i1):
                    if i - j not in h:
                        h[i - j] = f_s[pl.ds(pl.multiple_of(HF0 + row + (i - j) * FS, 8), 8), :]
                    p = h[i - j] * x
                    prev = acc[i - i0]
                    acc[i - i0] = p if prev is None else (prev + p if sign > 0 else prev - p)
                yield 2 * (i1 - max(i0, j))

        for i0, i1 in zip(BLOCKS[:-1], BLOCKS[1:]):
            k1 = [None] * (i1 - i0)
            yield from conv(0, i0, i1, k1, 1)
            zr = list(k1)
            yield from conv(2, i0, i1, zr, -1)
            yield from conv(1, i0, i1, k1, 1)
            for i in range(i1 - i0):
                z = jnp.concatenate([zr[i], k1[i]], axis=0).astype(BF16)
                z_s[c * NCH + i0 + i, pl.ds(pl.multiple_of(f8 * 16, 16), 16), :] = z
            yield i1 - i0

    qscale = float(DH ** -0.5 * np.log2(np.e))

    def attention(r0, src):
        def shifted(base, c, g, w):
            return src[pl.ds((base + c) * PT + HALO + 8 * g - DIL * w, 8), :]

        def scores(g):
            qs = [shifted(0, c, g, 0) for c in range(NC)]
            for w in range(WIN):
                acc = qs[0] * shifted(NC, 0, g, w)
                for c in range(1, NC):
                    acc = acc + qs[c] * shifted(NC, c, g, w)
                acc = acc + pltpu.roll(acc, 2 * NH, 1)
                acc = acc + pltpu.roll(acc, NH, 1)
                if 8 * g < DIL * w:
                    pos = r0 + 8 * g + lax.broadcasted_iota(jnp.int32, (8, L), 0)
                    acc = jnp.where(pos >= DIL * w, acc, -1e9)
                lg_s[pl.ds(8 * (g * WIN + w), 8), :] = acc
                yield 11

        def mix(g):
            logits = [lg_s[pl.ds(8 * (g * WIN + w), 8), :] for w in range(WIN)]
            m = logits[0]
            for w in range(1, WIN):
                m = jnp.maximum(m, logits[w])
            e = [jnp.exp2(l - m) for l in logits]
            den = e[0]
            for w in range(1, WIN):
                den = den + e[w]
            inv = pl.reciprocal(den, approx=True)
            inv = inv * (2.0 - den * inv)
            yield 30
            for c in range(NC):
                acc = e[0] * shifted(2 * NC, c, g, 0)
                for w in range(1, WIN):
                    acc = acc + e[w] * shifted(2 * NC, c, g, w)
                acc = acc * inv
                if g % 2 == 0:
                    half[c] = acc
                else:
                    o_s[c, pl.ds(r0 + 8 * (g - 1), 16), :] = jnp.concatenate(
                        [half[c], acc], axis=0).astype(BF16)
                yield 16

        groups = RT // 8
        half = [None] * NC
        for g in range(groups + LAG):
            if g < groups:
                yield from scores(g)
            if g >= LAG:
                yield from mix(g - LAG)

    def projections(jobs):
        def dot(job, ks):
            lhs_ref, r0, w_ref, n = job[:4]
            lhs = jnp.concatenate([lhs_ref[c, pl.ds(r0, RT), :] for c in ks], axis=1)
            if w_ref is wp_s:
                w = jnp.concatenate([pltpu.bitcast(w_ref[n * NC + c], BF16) for c in ks], axis=1)
                return lax.dot_general(lhs, w, _NT, preferred_element_type=F32)
            w = jnp.concatenate([pltpu.bitcast(w_ref[n * NC + c], BF16) for c in ks], axis=0)
            return jnp.dot(lhs, w, preferred_element_type=F32)

        rounds = []
        for g in range(0, len(jobs), 4):
            rounds += [[(job, dot(job, range(NC - 1)))] for job in jobs[g:g + 4]]
            rounds.append([(job, dot(job, [NC - 1])) for job in jobs[g:g + 4]])

        def stores():
            for i, rnd in enumerate(rounds):
                last = i % 5 == 4 or i == len(rounds) - 1
                for r in range(0, RT, SR):
                    for (_, _, _, _, dst, row, scale), y in rnd:
                        rows = pl.ds(row + r, SR)
                        yr = y[r:r + SR]
                        if last:
                            yr = yr + dst[rows, :]
                            yr = yr if scale is None else yr * scale
                        dst[rows, :] = yr
                    yield yr[SR - 8:]

        return stores(), len(rounds) * RT // SR

    def qkv_jobs(r0, dst):
        return [(q_s, r0, wp_s, n, dst, n * PT + HALO, qscale if n < NC else None)
                for n in range(3 * NC)]

    def out_jobs(r0):
        return [(o_s, r0, wop_s, n, b_s, n * BS + r0, None) for n in range(NC)]

    def chain(*gens):
        for g in gens:
            yield from g

    def weave(lead, steps, followers):
        done = [0] * len(followers)

        def advance(frac, anchor):
            for i, (gen, work, pace) in enumerate(followers):
                if anchor is not None and done[i] < frac * work:
                    pace(anchor)
                while done[i] < frac * work:
                    done[i] += next(gen)

        advance(PRE / (1 + PRE + POST), None)
        for i, anchor in enumerate(lead):
            advance(min((PRE + (i + 1) / steps) / (1 + PRE + POST), 1.0), anchor)
        advance(1.0, None)

    def gating(r0, n):
        for r in range(0, n, 16):
            rows = pl.ds(r0 + r, 16)
            dot = q_s[0, rows, :].astype(F32) * par_s[0, pl.ds(KS + 1, 1), :]
            for c in range(1, NC):
                dot = dot + q_s[c, rows, :].astype(F32) * par_s[c, pl.ds(KS + 1, 1), :]
            g = jnp.broadcast_to(jnp.sum(dot, axis=-1, keepdims=True), (16, L))
            g_s[rows, :] = 0.5 + 0.5 * jnp.tanh(0.5 * g) if TANH else jax.nn.sigmoid(g)
            yield 1

    def out_copy(i):
        rows = pl.ds(i * L, L)
        return pltpu.make_async_copy(out_s.at[rows, :], out_hbm.at[rows, :], out_sem.at[i])

    def finish(i):
        for c in range(NC):
            y = jnp.dot(inv_ref[...], z_s[c * NCH + i, pl.ds(0, 2 * L), :],
                        preferred_element_type=F32)
            for r in range(0, L, FR):
                rows = pl.ds(i * L + r, FR)
                b = b_s[pl.ds(c * BS + i * L + r, FR), :]
                a = q_s[c, rows, :].astype(F32) * y[r:r + FR]
                out_s[rows, c * L:(c + 1) * L] = (b + g_s[rows, :] * (a - b)).astype(BF16)
            yield y[L - 8:]

    attn_work = (RT // 8) * (11 * WIN + 30 + 16 * NC)

    def attn_stream(t, src):
        def pace(y):
            src[pl.ds(pl.multiple_of(PTOK + anywhere, 8), 8), :] = y
        return attention(pl.multiple_of(t * RT, RT), src), attn_work, pace

    def spec_stream(u0, n):
        def pace(y):
            f_s[pl.ds(pl.multiple_of(XTOK + anywhere, 8), 8), :] = y
        return chain(*[spectral(u0 + i) for i in range(n)]), n * (3 * NCH * (NCH + 1) + NCH), pace

    def gate_stream(r0, n=RT):
        def pace(y):
            par_s[NC, pl.ds(pl.multiple_of(anywhere, 8), 8), :] = y
        return gating(r0, n), n // 16, pace

    def part(stream, lo, hi):
        gen, work, pace = stream
        return gen, int(work * hi) // 8 * 8 - int(work * lo) // 8 * 8, pace

    def carry_halo(src, dst):
        for n in range(NC, 3 * NC):
            dst[pl.ds(n * PT, HALO), :] = src[pl.ds(n * PT + RT, HALO), :]

    anywhere = zero_ref[0]

    first = qkv_jobs(0, pa_s)
    w_cp[0].wait()
    permute_wqkv(0)
    wait(q_cp[0])
    weave(*projections(first[:4]), [])
    w_cp[1].wait()
    permute_wqkv(1)
    weave(*projections(first[4:7]), [])
    w_cp[2].wait()
    permute_wqkv(2)
    weave(*projections(first[7:]), [gate_stream(0)])

    wait(q_cp[1])
    carry_halo(pa_s, pb_s)
    weave(*projections(qkv_jobs(RT, pb_s)), [attn_stream(0, pa_s), gate_stream(RT)])

    wait(dft_cp + [hk_cp])
    gen, work, pace = attn_stream(1, pb_s)
    early = int(work * A1)
    weave(chain(*[filter_dft(c) for c in range(NC)]), 2 * NC * NCH, [(gen, early, pace)])

    for copies, j0, j1 in zip(kv_cp, KV_SPLIT[:-1], KV_SPLIT[1:]):
        wait(copies)
        weave(chain(*[signal_dft(j) for j in range(j0, j1)]), NC * (j1 - j0), [])

    wait([wo_cp] + q_cp[2])
    permute_wo()
    carry_halo(pb_s, pa_s)
    weave(*projections(qkv_jobs(2 * RT, pa_s) + out_jobs(0)),
          [spec_stream(0, U_FIRST), gate_stream(2 * RT), (gen, work - early - 40, pace)])
    for _ in gen:
        pass
    wait(q_cp[3])

    def phase(t, cur, nxt):
        row = lambda i: pl.multiple_of(i * RT, RT)
        carry_halo(cur, nxt)
        weave(*projections(out_jobs(row(t - 1)) + qkv_jobs(row(t + 1), nxt)),
              [attn_stream(t, cur), spec_stream(U_FIRST + (t - 2) * U_PHASE, U_PHASE)]
              + ([] if GT else [gate_stream(row(t + 1))]))

    @pl.loop(0, (NRT - 2) // 2)
    def _(i):
        phase(2 * i + 2, pa_s, pb_s)

        @pl.when(i < (NRT - 2) // 2 - 1)
        def _():
            phase(2 * i + 3, pb_s, pa_s)

    def tail(chunks, jobs, followers):
        lead, steps = projections(jobs) if jobs else ((), 0)
        weave(chain(lead, *[finish(i) for i in chunks]), steps + len(chunks) * NC, followers)

    gen, work, pace = attn_stream(NRT - 1, pb_s)
    tail(range(0, T1), out_jobs(S - 2 * RT), [(gen, int(work * A7), pace)] + ([gate_stream(3 * RT, GT * RT)] if GT else []))
    for i in range(0, T1):
        out_copy(i).start()
    tail(range(T1, T2), None, [(gen, work - int(work * A7) - 40, pace)]
         + ([gate_stream((3 + GT) * RT, (5 - GT) * RT)] if 0 < GT < 5 else []))
    for _ in gen:
        pass
    for i in range(T1, T2):
        out_copy(i).start()
    tail(range(T2, NCH - 2), out_jobs(S - RT), [])
    for i in range(T2, NCH - 2):
        out_copy(i).start()
    for i in range(NCH - 2, NCH):
        tail([i], None, [])
        out_copy(i).start()
    for i in range(NCH):
        out_copy(i).wait()


@jax.jit
def pallas_gated_mix__ssm_conv_h3__sliding_local_dilated__prompt_kernel(
    A_q: jax.Array,
    A_k: jax.Array,
    A_v: jax.Array,
    A_shift_k: jax.Array,
    A_ssm_k: jax.Array,
    A_ssm_D: jax.Array,
    B_x: jax.Array,
    B_wqkv: jax.Array,
    B_wo: jax.Array,
    gate_w: jax.Array,
):
    del B_x
    hbm = pl.BlockSpec(memory_space=pl.ANY)
    out = pl.pallas_call(
        _kernel,
        out_shape=jax.ShapeDtypeStruct((S, D), BF16),
        in_specs=[hbm] * 12,
        out_specs=hbm,
        scratch_shapes=[
            pltpu.VMEM((KS, D), BF16),
            pltpu.VMEM((D,), BF16),
            pltpu.VMEM((D,), BF16),
            pltpu.VMEM((2 * L, L), BF16),
            pltpu.VMEM((L, 2 * L), BF16),
            pltpu.SMEM((1,), jnp.int32),
            pltpu.VMEM((NC, S + PADB, L), BF16),
            pltpu.VMEM((S, D), BF16),
            pltpu.VMEM((S, D), BF16),
            pltpu.VMEM((D, S), BF16),
            pltpu.VMEM((3, D, D), BF16),
            pltpu.VMEM((D, D), BF16),
            pltpu.VMEM((3 * NC * NC, L // 2, L), U32),
            pltpu.VMEM((NC * NC, L // 2, L), U32),
            pltpu.VMEM((NC, D, L), F32),
            pltpu.VMEM((NC, 8 + S, L), F32),
            pltpu.VMEM((NC + 1, 8, L), F32),
            pltpu.VMEM((S, L), F32),
            pltpu.VMEM((NC * NCH, 2 * L + PADB, L), BF16),
            pltpu.VMEM((F_ROWS, L), F32),
            pltpu.VMEM((P_ROWS, L), F32),
            pltpu.VMEM((P_ROWS, L), F32),
            pltpu.VMEM((NC, S + PADB, L), BF16),
            pltpu.VMEM((NC * BS, L), F32),
            pltpu.VMEM((RT * WIN, L), F32),
            pltpu.VMEM((S, D), BF16),
            pltpu.SemaphoreType.DMA((N_IN_SEMS,)),
            pltpu.SemaphoreType.DMA((NCH,)),
        ],
        compiler_params=pltpu.CompilerParams(vmem_limit_bytes=110 * 1024 * 1024, flags=({os.environ['FLAG']: True} if 'FLAG' in os.environ else None)),
    )(
        A_q.reshape(S, D), A_k.reshape(S, D), A_v.reshape(S, D),
        A_shift_k.T, A_ssm_k, A_ssm_D, B_wqkv, B_wo, gate_w,
        _FWD, _INV, np.zeros((1,), np.int32),
    )
    return out.reshape(1, S, D)
```

```python
import jax
import jax.numpy as jnp
import numpy as np
from jax import lax
from jax.experimental import pallas as pl
from jax.experimental.pallas import tpu as pltpu

S = 2048
D = 640
NH = 32
DH = D // NH
WIN = 8
DIL = 2
KS = 4
L = 128
NC = D // L
NCH = S // L
NF8 = L // 8
HALO = 16
RT = 256
NRT = S // RT
F32 = jnp.float32
BF16 = jnp.bfloat16
U32 = jnp.uint32

SR = 32
LAG = 3
PRE, POST = 0.03, -0.015
BLOCKS = (0, 4, 8, 12, 16)
KV_SPLIT = (0, 8, 16)
U_PHASE = 13
U_FIRST = NC * NF8 - (NRT - 3) * U_PHASE
T1, T2 = 4, 11

FS = 3 * L + 16
XF0 = 0
HF0 = XF0 + NC * NCH * FS + 8
XTOK = HF0 + NC * NCH * FS
PT = HALO + RT + 8
PTOK = 3 * NC * PT
BS = S + 8
PADB = 16
N_IN_SEMS = 3 + 4 * NC + 1 + 2 * (len(KV_SPLIT) - 1) + 1 + 6


def _dft_matrices():
    n = np.arange(L)
    k = np.arange(L)
    ang = 2.0 * np.pi * (((4 * k[:, None] + 1) * n[None, :]) % (4 * L)) / (4 * L)
    fwd = np.concatenate([np.cos(ang), -np.sin(ang)], axis=0)
    inv = fwd.reshape(2, NF8, 8, L).transpose(1, 0, 2, 3).reshape(2 * L, L).T / L
    return fwd.astype(BF16), np.ascontiguousarray(inv).astype(BF16)


_FWD, _INV = _dft_matrices()
_NT = (((1,), (1,)), ((), ()))


def _kernel(q_hbm, k_hbm, v_hbm, shift_hbm, hk_hbm, ssmd_hbm, w_hbm, wo_hbm, gate_hbm,
            fwd_hbm, inv_hbm, zero_hbm, out_hbm,
            shift_ref, ssmd_ref, gate_ref, fwd_ref, inv_ref, zero_ref,
            q_s, k_s, v_s, hk_s, w_s, wo_s, wp_s, wop_s, tmp_s, kf_s, par_s, g_s,
            z_s, f_s, pa_s, pb_s, o_s, b_s, lg_s, out_s, in_sem, out_sem):
    sems = iter(range(N_IN_SEMS))

    def copy(src, dst):
        return pltpu.make_async_copy(src, dst, in_sem.at[next(sems)])

    w_cp = [copy(w_hbm.at[:, pl.ds(p * D, D)], w_s.at[p]) for p in range(3)]
    q_cp = [[copy(q_hbm.at[pl.ds(r0, n), pl.ds(c * L, L)], q_s.at[c, pl.ds(r0, n), :])
             for c in range(NC)]
            for r0, n in ((0, RT), (RT, RT), (2 * RT, RT), (3 * RT, S - 3 * RT))]
    hk_cp = copy(hk_hbm, hk_s)
    kv_cp = [[copy(src.at[pl.ds(j0 * L, (j1 - j0) * L), :], dst.at[pl.ds(j0 * L, (j1 - j0) * L), :])
              for src, dst in ((k_hbm, k_s), (v_hbm, v_s))]
             for j0, j1 in zip(KV_SPLIT[:-1], KV_SPLIT[1:])]
    wo_cp = copy(wo_hbm, wo_s)
    small_cp = [copy(zero_hbm, zero_ref), copy(shift_hbm, shift_ref), copy(ssmd_hbm, ssmd_ref),
                copy(gate_hbm, gate_ref)]
    dft_cp = [copy(fwd_hbm, fwd_ref), copy(inv_hbm, inv_ref)]
    for cp in (small_cp + [w_cp[0]] + q_cp[0] + w_cp[1:] + q_cp[1] + dft_cp
               + [hk_cp, wo_cp] + sum(kv_cp, []) + q_cp[2] + q_cp[3]):
        cp.start()

    def wait(copies):
        for cp in copies:
            cp.wait()

    wait(small_cp)
    taps = shift_ref[...].astype(F32)
    ssmd = ssmd_ref[...].astype(F32).reshape(1, D)
    gate = gate_ref[...].astype(F32).reshape(1, D)
    for c in range(NC):
        par_s[c, pl.ds(0, KS), :] = taps[:, c * L:(c + 1) * L]
        par_s[c, pl.ds(KS, 1), :] = ssmd[:, c * L:(c + 1) * L]
        par_s[c, pl.ds(KS + 1, 1), :] = gate[:, c * L:(c + 1) * L]
    for c in range(NC):
        kf_s[c, pl.ds(0, 8), :] = jnp.zeros((8, L), F32)
    for n in range(NC, 3 * NC):
        pa_s[pl.ds(n * PT, HALO), :] = jnp.zeros((HALO, L), F32)

    def filter_dft(c):
        prev = None
        for m in range(NCH):
            h = lax.dot_general(
                fwd_ref[...], hk_s[c * L:(c + 1) * L, m * L:(m + 1) * L], _NT, preferred_element_type=F32)
            hr, hi = h[:L], h[L:]
            if m == 0:
                hr = hr + par_s[c, pl.ds(KS, 1), :]
                a, b = hr, hi
            else:
                a, b = hr - prev[1], hi + prev[0]
            prev = (hr, hi)
            f_s[pl.ds(HF0 + (c * NCH + m) * FS, L), :] = a
            f_s[pl.ds(HF0 + (c * NCH + m) * FS + L, L), :] = b - a
            f_s[pl.ds(HF0 + (c * NCH + m) * FS + 2 * L, L), :] = a + b

    def signal_dft(j):
        for c in range(NC):
            rows, cols = pl.ds(j * L, L), slice(c * L, (c + 1) * L)
            k = k_s[rows, cols].astype(F32)
            kf_s[c, pl.ds(8 + j * L, L), :] = k
            ks = k * par_s[c, pl.ds(0, 1), :]
            for t in range(1, KS):
                ks = ks + kf_s[c, pl.ds(8 + j * L - t, L), :] * par_s[c, pl.ds(t, 1), :]
            kv = ks * v_s[rows, cols].astype(F32)
            x = jnp.dot(fwd_ref[...], kv.astype(BF16), preferred_element_type=F32)
            f_s[pl.ds(XF0 + (c * NCH + j) * FS, L), :] = x[:L] + x[L:]
            f_s[pl.ds(XF0 + (c * NCH + j) * FS + L, L), :] = x[:L]
            f_s[pl.ds(XF0 + (c * NCH + j) * FS + 2 * L, L), :] = x[L:]

    def head_major_to_dim_major(p):
        return jnp.concatenate([tmp_s[p, pl.ds(d, NH, stride=DH), :] for d in range(DH)], axis=0)

    def permute_wqkv(p):
        for rb in range(NC):
            tmp_s[rb, pl.ds(0, D), :] = w_s[p, rb * L:(rb + 1) * L, :].astype(F32).T
            wt = head_major_to_dim_major(rb).astype(BF16)
            for c in range(NC):
                wp_s[(p * NC + c) * NC + rb] = pltpu.bitcast(wt[c * L:(c + 1) * L], U32)

    def permute_wo():
        for c in range(NC):
            tmp_s[c, pl.ds(0, D), :] = wo_s[:, c * L:(c + 1) * L].astype(F32)
            wt = head_major_to_dim_major(c).astype(BF16)
            for rb in range(NC):
                wop_s[c * NC + rb] = pltpu.bitcast(wt[rb * L:(rb + 1) * L], U32)

    def spectral(u):
        c, f8 = u // NF8, u % NF8

        def conv(part, i0, i1, acc, sign):
            row = c * NCH * FS + part * L + f8 * 8
            h = {}
            for j in range(i1):
                x = f_s[pl.ds(pl.multiple_of(XF0 + row + j * FS, 8), 8), :]
                for i in range(max(i0, j), i1):
                    if i - j not in h:
                        h[i - j] = f_s[pl.ds(pl.multiple_of(HF0 + row + (i - j) * FS, 8), 8), :]
                    p = h[i - j] * x
                    prev = acc[i - i0]
                    acc[i - i0] = p if prev is None else (prev + p if sign > 0 else prev - p)
                yield 2 * (i1 - max(i0, j))

        for i0, i1 in zip(BLOCKS[:-1], BLOCKS[1:]):
            k1 = [None] * (i1 - i0)
            yield from conv(0, i0, i1, k1, 1)
            zr = list(k1)
            yield from conv(2, i0, i1, zr, -1)
            yield from conv(1, i0, i1, k1, 1)
            for i in range(i1 - i0):
                z = jnp.concatenate([zr[i], k1[i]], axis=0).astype(BF16)
                z_s[c * NCH + i0 + i, pl.ds(pl.multiple_of(f8 * 16, 16), 16), :] = z
            yield i1 - i0

    qscale = float(DH ** -0.5 * np.log2(np.e))

    def attention(r0, src):
        def shifted(base, c, g, w):
            return src[pl.ds((base + c) * PT + HALO + 8 * g - DIL * w, 8), :]

        def scores(g):
            qs = [shifted(0, c, g, 0) for c in range(NC)]
            for w in range(WIN):
                acc = qs[0] * shifted(NC, 0, g, w)
                for c in range(1, NC):
                    acc = acc + qs[c] * shifted(NC, c, g, w)
                acc = acc + pltpu.roll(acc, 2 * NH, 1)
                acc = acc + pltpu.roll(acc, NH, 1)
                if 8 * g < DIL * w:
                    pos = r0 + 8 * g + lax.broadcasted_iota(jnp.int32, (8, L), 0)
                    acc = jnp.where(pos >= DIL * w, acc, -1e9)
                lg_s[pl.ds(8 * (g * WIN + w), 8), :] = acc
                yield 11

        def mix(g):
            logits = [lg_s[pl.ds(8 * (g * WIN + w), 8), :] for w in range(WIN)]
            m = logits[0]
            for w in range(1, WIN):
                m = jnp.maximum(m, logits[w])
            e = [jnp.exp2(l - m) for l in logits]
            den = e[0]
            for w in range(1, WIN):
                den = den + e[w]
            inv = pl.reciprocal(den, approx=True)
            inv = inv * (2.0 - den * inv)
            yield 30
            for c in range(NC):
                acc = e[0] * shifted(2 * NC, c, g, 0)
                for w in range(1, WIN):
                    acc = acc + e[w] * shifted(2 * NC, c, g, w)
                acc = acc * inv
                if g % 2 == 0:
                    half[c] = acc
                else:
                    o_s[c, pl.ds(r0 + 8 * (g - 1), 16), :] = jnp.concatenate(
                        [half[c], acc], axis=0).astype(BF16)
                yield 16

        groups = RT // 8
        half = [None] * NC
        for g in range(groups + LAG):
            if g < groups:
                yield from scores(g)
            if g >= LAG:
                yield from mix(g - LAG)

    def projections(jobs):
        def dot(job, ks):
            lhs_ref, r0, w_ref, n = job[:4]
            lhs = jnp.concatenate([lhs_ref[c, pl.ds(r0, RT), :] for c in ks], axis=1)
            if w_ref is wp_s:
                w = jnp.concatenate([pltpu.bitcast(w_ref[n * NC + c], BF16) for c in ks], axis=1)
                return lax.dot_general(lhs, w, _NT, preferred_element_type=F32)
            w = jnp.concatenate([pltpu.bitcast(w_ref[n * NC + c], BF16) for c in ks], axis=0)
            return jnp.dot(lhs, w, preferred_element_type=F32)

        rounds = []
        for g in range(0, len(jobs), 4):
            rounds += [[(job, dot(job, range(NC - 1)))] for job in jobs[g:g + 4]]
            rounds.append([(job, dot(job, [NC - 1])) for job in jobs[g:g + 4]])

        def stores():
            for i, rnd in enumerate(rounds):
                last = i % 5 == 4 or i == len(rounds) - 1
                for r in range(0, RT, SR):
                    for (_, _, _, _, dst, row, scale), y in rnd:
                        rows = pl.ds(row + r, SR)
                        yr = y[r:r + SR]
                        if last:
                            yr = yr + dst[rows, :]
                            yr = yr if scale is None else yr * scale
                        dst[rows, :] = yr
                    yield yr[SR - 8:]

        return stores(), len(rounds) * RT // SR

    def qkv_jobs(r0, dst):
        return [(q_s, r0, wp_s, n, dst, n * PT + HALO, qscale if n < NC else None)
                for n in range(3 * NC)]

    def out_jobs(r0):
        return [(o_s, r0, wop_s, n, b_s, n * BS + r0, None) for n in range(NC)]

    def chain(*gens):
        for g in gens:
            yield from g

    def weave(lead, steps, followers):
        done = [0] * len(followers)

        def advance(frac, anchor):
            for i, (gen, work, pace) in enumerate(followers):
                if anchor is not None and done[i] < frac * work:
                    pace(anchor)
                while done[i] < frac * work:
                    done[i] += next(gen)

        advance(PRE / (1 + PRE + POST), None)
        for i, anchor in enumerate(lead):
            advance(min((PRE + (i + 1) / steps) / (1 + PRE + POST), 1.0), anchor)
        advance(1.0, None)

    def gating(r0):
        for r in range(0, RT, 16):
            rows = pl.ds(r0 + r, 16)
            dot = q_s[0, rows, :].astype(F32) * par_s[0, pl.ds(KS + 1, 1), :]
            for c in range(1, NC):
                dot = dot + q_s[c, rows, :].astype(F32) * par_s[c, pl.ds(KS + 1, 1), :]
            g = jnp.broadcast_to(jnp.sum(dot, axis=-1, keepdims=True), (16, L))
            g_s[rows, :] = 0.5 + 0.5 * jnp.tanh(0.5 * g)
            yield 1

    def out_copy(i):
        rows = pl.ds(i * L, L)
        return pltpu.make_async_copy(out_s.at[rows, :], out_hbm.at[rows, :], out_sem.at[i])

    def finish(i):
        for c in range(NC):
            y = jnp.dot(inv_ref[...], z_s[c * NCH + i, pl.ds(0, 2 * L), :],
                        preferred_element_type=F32)
            rows = pl.ds(i * L, L)
            b = b_s[pl.ds(c * BS + i * L, L), :]
            a = q_s[c, rows, :].astype(F32) * y
            out_s[rows, c * L:(c + 1) * L] = (b + g_s[rows, :] * (a - b)).astype(BF16)
            yield y[L - 8:]

    attn_work = (RT // 8) * (11 * WIN + 30 + 16 * NC)

    def attn_stream(t, src):
        def pace(y):
            src[pl.ds(pl.multiple_of(PTOK + anywhere, 8), 8), :] = y
        return attention(pl.multiple_of(t * RT, RT), src), attn_work, pace

    def spec_stream(u0, n):
        def pace(y):
            f_s[pl.ds(pl.multiple_of(XTOK + anywhere, 8), 8), :] = y
        return chain(*[spectral(u0 + i) for i in range(n)]), n * (3 * NCH * (NCH + 1) + NCH), pace

    def gate_stream(r0):
        def pace(y):
            par_s[NC, pl.ds(pl.multiple_of(anywhere, 8), 8), :] = y
        return gating(r0), RT // 16, pace

    def carry_halo(src, dst):
        for n in range(NC, 3 * NC):
            dst[pl.ds(n * PT, HALO), :] = src[pl.ds(n * PT + RT, HALO), :]

    anywhere = zero_ref[0]

    first = qkv_jobs(0, pa_s)
    w_cp[0].wait()
    permute_wqkv(0)
    wait(q_cp[0])
    weave(*projections(first[:4]), [])
    w_cp[1].wait()
    permute_wqkv(1)
    weave(*projections(first[4:7]), [])
    w_cp[2].wait()
    permute_wqkv(2)
    weave(*projections(first[7:]), [gate_stream(0)])

    wait(q_cp[1])
    carry_halo(pa_s, pb_s)
    weave(*projections(qkv_jobs(RT, pb_s)), [attn_stream(0, pa_s), gate_stream(RT)])

    wait(dft_cp + [hk_cp, wo_cp])
    permute_wo()
    for c in range(NC):
        filter_dft(c)

    for copies, j0, j1 in zip(kv_cp, KV_SPLIT[:-1], KV_SPLIT[1:]):
        wait(copies)
        for j in range(j0, j1):
            signal_dft(j)

    wait(q_cp[2])
    carry_halo(pb_s, pa_s)
    weave(*projections(qkv_jobs(2 * RT, pa_s) + out_jobs(0)),
          [spec_stream(0, U_FIRST), gate_stream(2 * RT), attn_stream(1, pb_s)])
    wait(q_cp[3])

    def phase(t, cur, nxt):
        row = lambda i: pl.multiple_of(i * RT, RT)
        carry_halo(cur, nxt)
        weave(*projections(out_jobs(row(t - 1)) + qkv_jobs(row(t + 1), nxt)),
              [attn_stream(t, cur), spec_stream(U_FIRST + (t - 2) * U_PHASE, U_PHASE),
               gate_stream(row(t + 1))])

    @pl.loop(0, (NRT - 2) // 2)
    def _(i):
        phase(2 * i + 2, pa_s, pb_s)

        @pl.when(i < (NRT - 2) // 2 - 1)
        def _():
            phase(2 * i + 3, pb_s, pa_s)

    def tail(chunks, jobs, followers):
        lead, steps = projections(jobs) if jobs else ((), 0)
        weave(chain(lead, *[finish(i) for i in chunks]), steps + len(chunks) * NC, followers)

    gen, work, pace = attn_stream(NRT - 1, pb_s)
    tail(range(0, T1), out_jobs(S - 2 * RT), [(gen, work // 2, pace)])
    for i in range(0, T1):
        out_copy(i).start()
    tail(range(T1, T2), None, [(gen, work // 2 - 40, pace)])
    for _ in gen:
        pass
    for i in range(T1, T2):
        out_copy(i).start()
    tail(range(T2, NCH - 2), out_jobs(S - RT), [])
    for i in range(T2, NCH - 2):
        out_copy(i).start()
    for i in range(NCH - 2, NCH):
        tail([i], None, [])
        out_copy(i).start()
    for i in range(NCH):
        out_copy(i).wait()


@jax.jit
def pallas_gated_mix__ssm_conv_h3__sliding_local_dilated__prompt_kernel(
    A_q: jax.Array,
    A_k: jax.Array,
    A_v: jax.Array,
    A_shift_k: jax.Array,
    A_ssm_k: jax.Array,
    A_ssm_D: jax.Array,
    B_x: jax.Array,
    B_wqkv: jax.Array,
    B_wo: jax.Array,
    gate_w: jax.Array,
):
    del B_x
    hbm = pl.BlockSpec(memory_space=pl.ANY)
    out = pl.pallas_call(
        _kernel,
        out_shape=jax.ShapeDtypeStruct((S, D), BF16),
        in_specs=[hbm] * 12,
        out_specs=hbm,
        scratch_shapes=[
            pltpu.VMEM((KS, D), BF16),
            pltpu.VMEM((D,), BF16),
            pltpu.VMEM((D,), BF16),
            pltpu.VMEM((2 * L, L), BF16),
            pltpu.VMEM((L, 2 * L), BF16),
            pltpu.SMEM((1,), jnp.int32),
            pltpu.VMEM((NC, S + PADB, L), BF16),
            pltpu.VMEM((S, D), BF16),
            pltpu.VMEM((S, D), BF16),
            pltpu.VMEM((D, S), BF16),
            pltpu.VMEM((3, D, D), BF16),
            pltpu.VMEM((D, D), BF16),
            pltpu.VMEM((3 * NC * NC, L // 2, L), U32),
            pltpu.VMEM((NC * NC, L // 2, L), U32),
            pltpu.VMEM((NC, D + 24, L), F32),
            pltpu.VMEM((NC, 8 + S, L), F32),
            pltpu.VMEM((NC + 1, 8, L), F32),
            pltpu.VMEM((S, L), F32),
            pltpu.VMEM((NC * NCH, 2 * L + PADB, L), BF16),
            pltpu.VMEM((XTOK + 8, L), F32),
            pltpu.VMEM((PTOK + 8, L), F32),
            pltpu.VMEM((PTOK + 8, L), F32),
            pltpu.VMEM((NC, S + PADB, L), BF16),
            pltpu.VMEM((NC * BS, L), F32),
            pltpu.VMEM((RT * WIN, L), F32),
            pltpu.VMEM((S, D), BF16),
            pltpu.SemaphoreType.DMA((N_IN_SEMS,)),
            pltpu.SemaphoreType.DMA((NCH,)),
        ],
        compiler_params=pltpu.CompilerParams(vmem_limit_bytes=110 * 1024 * 1024),
    )(
        A_q.reshape(S, D), A_k.reshape(S, D), A_v.reshape(S, D),
        A_shift_k.T, A_ssm_k, A_ssm_D, B_wqkv, B_wo, gate_w,
        _FWD, _INV, np.zeros((1,), np.int32),
    )
    return out.reshape(1, S, D)
```
